```python
import jax
import jax.numpy as jnp

def _softmax(x, axis=-1):
    return jax.nn.softmax(x, axis=axis)
def _gelu(x):
    return jax.nn.gelu(x, approximate=True)
def _silu(x):
    return jax.nn.silu(x)
def _sigmoid(x):
    return jax.nn.sigmoid(x)
def _layernorm(x, axis=-1, eps=1e-5):
    m = jnp.mean(x, axis=axis, keepdims=True)
    v = jnp.var(x, axis=axis, keepdims=True)
    return (x - m) / jnp.sqrt(v + eps)
def _scatter_add(tgt, idx, src, axis=0):
    return tgt.at[idx].add(src)
def _segment_sum(src, seg, n):
    return jax.ops.segment_sum(src, seg, n)
class _Rng:
    def __init__(self, key):
        self._k = key
    def _next(self):
        self._k, sub = jax.random.split(self._k)
        return sub
    def normal(self, shape):
        return jax.random.normal(self._next(), shape, dtype=jnp.bfloat16)
    def randint(self, lo, hi, shape):
        return jax.random.randint(self._next(), shape, lo, hi, dtype=jnp.int32)
    def uniform(self, shape, lo=0.0, hi=1.0):
        return jax.random.uniform(self._next(), shape, jnp.bfloat16, lo, hi)
    def permutation(self, n):
        return jax.random.permutation(self._next(), n)


kernel_name = 'interleave_layers__compressed_kv_cla__moe_arch_mod__decode'

def setup_inputs():
    _rng = _Rng(jax.random.key(int.from_bytes(__import__("os").urandom(4), "little")))
    _w = (lambda a: (lambda t: t.astype(jnp.bfloat16) if jnp.issubdtype(t.dtype, jnp.floating) else t)(jnp.asarray(a)))
    def _A_setup():
        B, H, Sq, Sk, D, M = 1, 32, 1, 4096, 128, 640
        Dc = 4 * D
        return {
            "x": _w((lambda *s: _rng.normal(s) * 0.05)(B, Sq, M)),
            "c_kv": _w((lambda *s: _rng.normal(s) * 0.05)(B, Sk, Dc)),
            "w_q": _w((lambda *s: _rng.normal(s) * 0.05)(M, H, D) * (M ** -0.5)),
            "w_uk": _w((lambda *s: _rng.normal(s) * 0.05)(Dc, H, D) * (Dc ** -0.5)),
            "w_uv": _w((lambda *s: _rng.normal(s) * 0.05)(Dc, H, D) * (Dc ** -0.5)),
            "w_o": _w((lambda *s: _rng.normal(s) * 0.05)(H, D, M) * ((H * D) ** -0.5)),
        }
    _A_in = _A_setup()

    def _B_setup():
        B, S, D, F, C = 1, 1, 640, 1728, 1
        return {
            "x": _w((lambda *s: _rng.normal(s) * 0.05)(B, S, D)),
            "w_r": _w((lambda *s: _rng.normal(s) * 0.05)(D)),
            "w_gate": _w((lambda *s: _rng.normal(s) * 0.05)(D, F)),
            "w_up": _w((lambda *s: _rng.normal(s) * 0.05)(D, F)),
            "w_down": _w((lambda *s: _rng.normal(s) * 0.05)(F, D)),
        }
    _B_in = _B_setup()

    return {
        "A_x": _A_in["x"],
        "A_c_kv": _A_in["c_kv"],
        "A_w_q": _A_in["w_q"],
        "A_w_uk": _A_in["w_uk"],
        "A_w_uv": _A_in["w_uv"],
        "A_w_o": _A_in["w_o"],
        "B_x": _B_in["x"],
        "B_w_r": _B_in["w_r"],
        "B_w_gate": _B_in["w_gate"],
        "B_w_up": _B_in["w_up"],
        "B_w_down": _B_in["w_down"],
    }

def reference(A_x, A_c_kv, A_w_q, A_w_uk, A_w_uv, A_w_o, B_x, B_w_r, B_w_gate, B_w_up, B_w_down):
    def _A_ref(x, c_kv, w_q, w_uk, w_uv, w_o):
        B, Sq, M = x.shape[0], x.shape[1], x.shape[2]
        Sk = c_kv.shape[1]
        H, D = w_q.shape[1], w_q.shape[2]
        q = jnp.einsum("bqm,mhd->bhqd", x, w_q)
        k = jnp.einsum("bkc,chd->bhkd", c_kv, w_uk)
        v = jnp.einsum("bkc,chd->bhkd", c_kv, w_uv)
        scores = jnp.einsum("bhqd,bhkd->bhqk", q, k) * (D ** -0.5)
        off = Sk - Sq
        qi = jnp.arange(Sq)[:, None]
        kj = jnp.arange(Sk)[None, :]
        cmask = kj <= (qi + off)
        scores = jnp.where(cmask[None, None], scores, -1e9)
        p = _softmax(scores, axis=-1)
        ctx = jnp.einsum("bhqk,bhkd->bhqd", p, v)
        return jnp.einsum("bhqd,hdm->bqm", ctx, w_o)

    def _B_ref(x, w_r, w_gate, w_up, w_down):
        B, S, D = x.shape
        C = 1
        r = x @ w_r
        idx = jnp.argsort(-r, axis=-1)[:, :C]
        idx_e = jnp.repeat(idx.reshape(B, C, 1), D, axis=2)
        x_sel = jnp.take_along_axis(x, idx_e, axis=1)
        g = _silu(x_sel @ w_gate)
        u = x_sel @ w_up
        y = (g * u) @ w_down
        r_sel = _sigmoid(jnp.take_along_axis(r, idx, axis=1))
        y = y * r_sel.reshape(B, C, 1)
        b_off = (jnp.arange(B) * S).reshape(B, 1)
        flat_idx = (idx + b_off).reshape(B * C)
        zero = (x * 0.0).reshape(B * S, D)
        upd = _scatter_add(zero, flat_idx, y.reshape(B * C, D), axis=0)
        return x + upd.reshape(B, S, D)

    x = A_x
    x = x + _A_ref(_layernorm(x, axis=-1), A_c_kv, A_w_q, A_w_uk, A_w_uv, A_w_o)
    x = x + _B_ref(_layernorm(x, axis=-1), B_w_r, B_w_gate, B_w_up, B_w_down)
    x = x + _A_ref(_layernorm(x, axis=-1), A_c_kv, A_w_q, A_w_uk, A_w_uv, A_w_o)
    x = x + _B_ref(_layernorm(x, axis=-1), B_w_r, B_w_gate, B_w_up, B_w_down)
    return x
```

```python
import functools
import numpy as np
import jax
import jax.numpy as jnp
from jax import lax
import jax.experimental.pallas as pl
import jax.experimental.pallas.tpu as pltpu

M, H, D, DC, SK, F = 640, 32, 128, 512, 4096, 1728
NMB = M // 128
NCB = DC // 128
NKB = SK // 128
NFB = F // 128
FREM = F - NFB * 128
LOG2E = 1.4426950408889634
BF = jnp.bfloat16
F32 = jnp.float32
U32 = jnp.uint32


def _dot(a, b):
    return jnp.dot(a, b, preferred_element_type=F32)


def _tile(ref_u32, r0):
    return pltpu.bitcast(ref_u32[pl.ds(r0, 64), :], BF)


def _iota(shape, ax):
    return lax.broadcasted_iota(jnp.int32, shape, ax)


def _pack_rows(v):
    return pltpu.bitcast(v.astype(BF), U32)


def _layernorm(x):
    s = x[0]
    for b in range(1, NMB):
        s = s + x[b]
    mean = jnp.sum(s, axis=1, keepdims=True) * (1.0 / M)
    xc = [xb - mean for xb in x]
    v = xc[0] * xc[0]
    for b in range(1, NMB):
        v = v + xc[b] * xc[b]
    var = jnp.sum(v, axis=1, keepdims=True) * (1.0 / M)
    inv = lax.rsqrt(var + 1e-5)
    return [xb * inv for xb in xc]


def _rep16(v):
    return jnp.concatenate([v, v], axis=0).astype(BF)


def build(opts=None):
    opts = dict(opts or {})
    WO_RC = opts.get('wo_rc', 8)
    WD_RC = opts.get('wd_rc', 4)
    scoped = opts.get('scoped', False)
    only_pass2 = opts.get('only_pass2', 0)

    def scope(name):
        if scoped:
            return jax.named_scope(name)
        import contextlib
        return contextlib.nullcontext()

    def kernel(x_hbm, wr_hbm, wq_hbm, wuk_hbm, ckv_hbm, wuv_hbm, wo_hbm, wg_hbm, wu_hbm, wd_hbm,
               o_ref,
               xb, wrb, wq, wuk, ukT, ckv, ckvT, wuv, wo, wg, wu, guT, wd, s_scr, sems):
        def cp(src, dst, s):
            return pltpu.make_async_copy(src, dst, sems.at[s])
        g_q = [cp(wq_hbm, wq, 0), cp(x_hbm, xb, 0), cp(wr_hbm, wrb, 0)]
        g_uk = [cp(wuk_hbm, wuk, 1)]
        g_ckv = [cp(ckv_hbm.at[:, pl.ds(j * 128, 128)], ckv.at[pl.ds(j * SK, SK)], 2) for j in range(NCB)]
        g_uv = [cp(wuv_hbm, wuv, 3)]
        g_g = [cp(wg_hbm, wg, 4)]
        g_u = [cp(wu_hbm, wu, 5)]
        g_o = []
        for r in range(WO_RC):
            n = SK // WO_RC
            for j in range(NMB):
                g_o.append(cp(wo_hbm.at[pl.ds(r * n, n), pl.ds(j * 128, 128)], wo.at[pl.ds(j * SK + r * n, n)], 6))
        FSPLIT = opts.get('fsplit', 11)
        g_d1, g_d2 = [], []
        nrc = WD_RC - 1
        bounds = [(FSPLIT * j // nrc) * 128 for j in range(nrc + 1)] + [F]
        for r in range(WD_RC):
            a, b = bounds[r], bounds[r + 1]
            for j in range(NMB):
                last = r == WD_RC - 1
                (g_d2 if last else g_d1).append(
                    cp(wd_hbm.at[pl.ds(a, b - a), pl.ds(j * 128, 128)], wd.at[pl.ds(j * F + a, b - a)], 8 if last else 7))
        for grp in (g_q, g_uk, g_ckv, g_uv, g_g, g_u, g_o, g_d1, g_d2):
            for c in grp:
                c.start()

        def wait(grp):
            for c in grp:
                c.wait()

        lane = _iota((8, 128), 1)
        sub = _iota((8, 128), 0)
        h16 = lane % 16
        XM = jnp.where(h16 == 2 * sub, np.uint32(0x0000FFFF),
                       jnp.where(h16 == 2 * sub + 1, np.uint32(0xFFFF0000), np.uint32(0)))
        idx16 = lane // 16
        PM = jnp.where(lane % 2 == 0, np.uint32(0x0000FFFF), np.uint32(0xFFFF0000))
        idx2 = lane // 2

        wq_u = wq.bitcast(U32)
        wuk_u = wuk.bitcast(U32)
        wuv_u = wuv.bitcast(U32)
        ckv_u = ckv.bitcast(U32)
        ckvT_u = ckvT.bitcast(U32)
        wo_u = wo.bitcast(U32)
        guT_u = guT.bitcast(U32)
        wd_u = wd.bitcast(U32)

        def xtrick(srcs, w_u, ngroups):
            acc = [None, None]
            for g in range(ngroups):
                blk, r = divmod(g, 16)
                idx = idx16 + 8 * r
                shared = srcs[0][blk] is srcs[1][blk]
                l0 = None
                for hh in range(2):
                    if hh == 0 or not shared:
                        l0 = pltpu.bitcast(jnp.take_along_axis(srcs[hh][blk], idx, axis=1) & XM, BF)
                    rows = [w_u[pl.ds((8 * g + j) * 16 + 8 * hh, 8), :] for j in range(8)]
                    t = pltpu.bitcast(jnp.concatenate(rows, axis=0), BF)
                    o = _dot(l0, t)
                    acc[hh] = o if acc[hh] is None else acc[hh] + o
            return acc

        def stage_a(xn):
            srcs = []
            for b in range(NMB):
                u = pltpu.bitcast(xn[b].astype(BF).astype(F32), U32)
                srcs.append(u | (u >> 16))
            return xtrick([srcs, srcs], wq_u, M // 8)

        def relayout_uk():
            for hp in range(16):
                for cb in range(NCB):
                    s = wuk_u[pl.ds(128 * cb * 16 + hp, 128, stride=16), :]
                    ukT[pl.ds((hp * NCB + cb) * 128, 128), :] = s.T

        def stage_b(q):
            qabs = [[None] * NCB for _ in range(2)]
            for hh in range(2):
                qp = _pack_rows(q[hh])
                L = [jnp.take_along_axis(qp, idx2 + 64 * kh, axis=1) & PM for kh in range(2)]
                for hp8 in range(8):
                    hp = hh * 8 + hp8
                    Lm = [pltpu.bitcast(jnp.where(sub == hp8, L[kh], np.uint32(0)), BF) for kh in range(2)]
                    for cb in range(NCB):
                        for kh in range(2):
                            o = _dot(Lm[kh], _tile(ukT, (hp * NCB + cb) * 128 + 64 * kh))
                            qabs[hh][cb] = o if qabs[hh][cb] is None else qabs[hh][cb] + o
            return qabs

        def transpose_ckv():
            for cb in range(NCB):
                for kb in range(NKB):
                    t = ckv[pl.ds(cb * SK + kb * 128, 128), :]
                    ckvT[pl.ds((cb * NKB + kb) * 128, 128), :] = t.T

        def stage_cd(qabs):
            lhs = [jnp.concatenate([qabs[0][cb], qabs[1][cb]], axis=0).astype(BF) for cb in range(NCB)]
            mx = None
            for kb in range(NKB):
                s = None
                for cb in range(NCB):
                    o = _dot(lhs[cb], _tile(ckvT_u, (cb * NKB + kb) * 64))
                    s = o if s is None else s + o
                s_scr[:, kb * 128:(kb + 1) * 128] = s
                mx = s if mx is None else jnp.maximum(mx, s)
            m = jnp.max(mx, axis=1, keepdims=True)
            c = (D ** -0.5) * LOG2E
            acc = [None] * NCB
            l = None
            for kb in range(NKB):
                p = jnp.exp2((s_scr[:, kb * 128:(kb + 1) * 128] - m) * c)
                l = p if l is None else l + p
                pb = p.astype(BF)
                for cb in range(NCB):
                    o = _dot(pb, _tile(ckv_u, cb * (SK // 2) + kb * 64))
                    acc[cb] = o if acc[cb] is None else acc[cb] + o
            linv = 1.0 / jnp.sum(l, axis=1, keepdims=True)
            return [a * linv for a in acc]

        def stage_e(ctxc):
            srcs = [[_pack_rows(ctxc[cb][16 * hh:16 * hh + 16]) for cb in range(NCB)] for hh in range(2)]
            return xtrick(srcs, wuv_u, DC // 8)

        def stage_f(ctx):
            acc = [None] * NMB
            for h in range(H):
                hh, r = divmod(h, 16)
                L = jnp.broadcast_to(ctx[hh][r:r + 1, :], (16, 128)).astype(BF)
                for mb in range(NMB):
                    o = _dot(L, _tile(wo_u, mb * (SK // 2) + h * 64))
                    acc[mb] = o if acc[mb] is None else acc[mb] + o
            return [a[0:8] for a in acc]

        def gu_index(which, fb, mb):
            return (which * NFB + fb) * NMB + mb

        def transpose_gu(which, src):
            for fb in range(NFB):
                for mb in range(NMB):
                    t = src[pl.ds(fb * 128, 128), pl.ds(mb * 128, 128)]
                    guT[pl.ds(gu_index(which, fb, mb) * 128, 128), :] = t.T

        def transpose_gu_last():
            for mb in range(NMB):
                t = jnp.concatenate([wg[pl.ds(NFB * 128, FREM), pl.ds(mb * 128, 128)],
                                     wu[pl.ds(NFB * 128, FREM), pl.ds(mb * 128, 128)]], axis=0)
                guT[pl.ds((2 * NFB * NMB + mb) * 128, 128), :] = t.T

        def silu(g):
            return g / (1.0 + jnp.exp(-g))

        def stage_g(xn):
            L = [_rep16(xn[b]) for b in range(NMB)]
            hs = []
            for fb in range(NFB):
                gu = []
                for which in range(2):
                    a = None
                    for mb in range(NMB):
                        o = _dot(L[mb], _tile(guT_u, gu_index(which, fb, mb) * 64))
                        a = o if a is None else a + o
                    gu.append(a[0:8])
                hs.append(silu(gu[0]) * gu[1])
            a = None
            for mb in range(NMB):
                o = _dot(L[mb], _tile(guT_u, (2 * NFB * NMB + mb) * 64))
                a = o if a is None else a + o
            a = a[0:8]
            sw = pltpu.roll(a, 64, axis=1)
            g = jnp.where(lane < 64, a, sw)
            u = jnp.where(lane < 64, sw, a)
            hs.append(silu(g) * u)
            return hs

        def stage_h(hs, fbs, acc, last):
            for fb in fbs:
                L = _rep16(hs[fb])
                for mb in range(NMB):
                    o = _dot(L, _tile(wd_u, mb * (F // 2) + fb * 64))
                    acc[mb] = o if acc[mb] is None else acc[mb] + o
            if last:
                hl = hs[NFB]
                z = jnp.zeros_like(hl)
                ev = jnp.where(lane < 64, hl, z)
                od = jnp.where(lane < 64, z, hl)
                rowsA = jnp.where(sub % 2 == 0, ev, od)
                L = _rep16(rowsA)
                r0 = NFB * 64
                for mb in range(0, NMB, 2):
                    mb2 = min(mb + 1, NMB - 1)
                    t = jnp.concatenate([wd_u[pl.ds(mb * (F // 2) + r0, 32), :], wd_u[pl.ds(mb2 * (F // 2) + r0, 32), :]], axis=0)
                    o = _dot(L, pltpu.bitcast(t, BF))[0:8]
                    o0 = jnp.broadcast_to(o[0:1], (8, 128))
                    acc[mb] = acc[mb][0:8] + o0
                    if mb2 != mb:
                        acc[mb2] = acc[mb2][0:8] + jnp.broadcast_to(o[1:2], (8, 128))
            return acc

        def one_pass(x, first):
            xn = _layernorm(x)
            if first:
                pass
            with scope('a'):
                q = stage_a(xn)
            if first:
                wait(g_uk)
                relayout_uk()
            with scope('b'):
                qabs = stage_b(q)
            if first:
                wait(g_ckv)
                transpose_ckv()
            with scope('cd'):
                ctxc = stage_cd(qabs)
            if first:
                wait(g_uv)
            with scope('e'):
                ctx = stage_e(ctxc)
            if first:
                wait(g_g)
                transpose_gu(0, wg)
                wait(g_u)
                transpose_gu(1, wu)
                transpose_gu_last()
                wait(g_o)
            with scope('f'):
                att = stage_f(ctx)
            x1 = [x[b] + att[b] for b in range(NMB)]
            xn1 = _layernorm(x1)
            rr = xn1[0] * wr_rows[0]
            for b in range(1, NMB):
                rr = rr + xn1[b] * wr_rows[b]
            r = jnp.sum(rr, axis=1, keepdims=True)
            sig = 1.0 / (1.0 + jnp.exp(-r))
            with scope('g'):
                hs = stage_g(xn1)
            acc = [None] * NMB
            with scope('h'):
                if first:
                    wait(g_d1)
                    acc = stage_h(hs, range(FSPLIT), acc, False)
                    wait(g_d2)
                    acc = stage_h(hs, range(FSPLIT, NFB), acc, True)
                else:
                    acc = stage_h(hs, range(NFB), acc, True)
            return [x1[b] + xn1[b] + acc[b] * sig for b in range(NMB)]

        wait(g_q)
        xrow = xb[0].astype(F32)
        x = [jnp.broadcast_to(xrow[:, b * 128:(b + 1) * 128], (8, 128)) for b in range(NMB)]
        wrf = wrb[...].astype(F32)
        wr_rows = [jnp.broadcast_to(wrf[b:b + 1, :], (8, 128)) for b in range(NMB)]
        x = one_pass(x, True)
        for _ in range(1 + only_pass2):
            x = one_pass(x, False)
        out = jnp.concatenate([xb_[0:1] for xb_ in x], axis=1)
        o_ref[...] = out.astype(BF).reshape(1, 1, M)

    scratch = [
        pltpu.VMEM((1, 1, M), BF),
        pltpu.VMEM((NMB, 128), BF),
        pltpu.VMEM((M * H, D), BF),
        pltpu.VMEM((DC * H, D), BF),
        pltpu.VMEM((DC * H // 2, D), U32),
        pltpu.VMEM((NCB * SK, 128), BF),
        pltpu.VMEM((NCB * SK, 128), BF),
        pltpu.VMEM((DC * H, D), BF),
        pltpu.VMEM((NMB * SK, 128), BF),
        pltpu.VMEM((F, M), BF),
        pltpu.VMEM((F, M), BF),
        pltpu.VMEM(((2 * NFB * NMB + NMB) * 128, 128), BF),
        pltpu.VMEM((NMB * F, 128), BF),
        pltpu.VMEM((H, SK), F32),
        pltpu.SemaphoreType.DMA((9,)),
    ]

    def fn(A_x, A_c_kv, A_w_q, A_w_uk, A_w_uv, A_w_o, B_x, B_w_r, B_w_gate, B_w_up, B_w_down):
        return pl.pallas_call(
            kernel,
            out_shape=jax.ShapeDtypeStruct((1, 1, M), BF),
            in_specs=[pl.BlockSpec(memory_space=pltpu.HBM)] * 10,
            out_specs=pl.BlockSpec(memory_space=pltpu.VMEM),
            scratch_shapes=scratch,
            compiler_params=pltpu.CompilerParams(vmem_limit_bytes=100 * 1024 * 1024),
        )(A_x, B_w_r.reshape(NMB, 128), A_w_q.reshape(M * H, D), A_w_uk.reshape(DC * H, D),
          A_c_kv.reshape(SK, DC), A_w_uv.reshape(DC * H, D), A_w_o.reshape(H * D, M),
          B_w_gate.T, B_w_up.T, B_w_down)
    return fn


@jax.jit
def pallas_interleave_layers__compressed_kv_cla__moe_arch_mod__decode_kernel(
    A_x: jax.Array,
    A_c_kv: jax.Array,
    A_w_q: jax.Array,
    A_w_uk: jax.Array,
    A_w_uv: jax.Array,
    A_w_o: jax.Array,
    B_x: jax.Array,
    B_w_r: jax.Array,
    B_w_gate: jax.Array,
    B_w_up: jax.Array,
    B_w_down: jax.Array,
):
    fn = build({})
    return fn(A_x, A_c_kv, A_w_q, A_w_uk, A_w_uv, A_w_o, B_x, B_w_r, B_w_gate, B_w_up, B_w_down)
```

```python
import functools
import contextlib
import numpy as np
import jax
import jax.numpy as jnp
from jax import lax
import jax.experimental.pallas as pl
import jax.experimental.pallas.tpu as pltpu

M, H, D, DC, SK, F = 640, 32, 128, 512, 4096, 1728
NMB = M // 128
NCB = DC // 128
NKB = SK // 128
NFB = F // 128
FREM = F - NFB * 128
LOG2E = 1.4426950408889634
EPS = 1e-5
BF = jnp.bfloat16
F32 = jnp.float32
U32 = jnp.uint32


def _dot(a, b):
    return jnp.dot(a, b, preferred_element_type=F32)


def _tile(ref_u32, r0):
    return pltpu.bitcast(ref_u32[pl.ds(r0, 64), :], BF)


def _iota(shape, ax):
    return lax.broadcasted_iota(jnp.int32, shape, ax)


def _pack_rows(v):
    return pltpu.bitcast(v.astype(BF), U32)


def _stats(x):
    s = x[0]
    for b in range(1, NMB):
        s = s + x[b]
    mean = jnp.sum(s, axis=1, keepdims=True) * (1.0 / M)
    xc = [xb - mean for xb in x]
    v = xc[0] * xc[0]
    for b in range(1, NMB):
        v = v + xc[b] * xc[b]
    var = jnp.sum(v, axis=1, keepdims=True) * (1.0 / M)
    return mean, lax.rsqrt(var + EPS)


def _rep16(v):
    return jnp.concatenate([v, v], axis=0).astype(BF)


def unpack(w):
    lo = pltpu.bitcast(w << 16, F32)
    hi = pltpu.bitcast(w & np.uint32(0xFFFF0000), F32)
    return lo, hi


def _acc(a, o):
    return o if a is None else a + o


def build(opts=None):
    opts = dict(opts or {})
    WO_RC = opts.get('wo_rc', 8)
    WD_RC = opts.get('wd_rc', 12)
    WD_SPLIT = opts.get('wd_split', 9)
    NA = opts.get('na', 8)
    NB2 = opts.get('nb2', 8)
    G1 = opts.get('g1', 3)
    scoped = opts.get('scoped', False)
    extra = opts.get('extra', 0)

    def scope(name):
        if scoped:
            return jax.named_scope(name)
        import contextlib
        return contextlib.nullcontext()

    def kernel(x_hbm, wr_hbm, wq_hbm, wuk_hbm, ckv_hbm, wuv_hbm, wo_hbm, wg_hbm, wu_hbm, wd_hbm,
               o_ref,
               xb, wrb, wq, wuk, ukT, ckv, ckvT, wuv, wo, wg, wu, guT, wd, s_scr, cs_scr, sems):
        def cp(src, dst, s):
            return pltpu.make_async_copy(src, dst, sems.at[s])
        g_q = [cp(wq_hbm, wq, 0), cp(x_hbm, xb, 0), cp(wr_hbm, wrb, 0)]
        g_uk = [cp(wuk_hbm, wuk, 1)]
        g_ckv = [cp(ckv_hbm.at[:, pl.ds(j * 128, 128)], ckv.at[pl.ds(j * SK, SK)], 2) for j in range(NCB)]
        g_uv = [cp(wuv_hbm, wuv, 0)]
        g_g = [cp(wg_hbm, wg, 1)]
        g_u = [cp(wu_hbm, wu, 2)]
        NH1 = opts.get('nh1', 24)
        g_o1, g_o2 = [], []
        for r in range(WO_RC):
            n = SK // WO_RC
            for j in range(NMB):
                p1 = r * n < NH1 * D
                (g_o1 if p1 else g_o2).append(
                    cp(wo_hbm.at[pl.ds(r * n, n), pl.ds(j * 128, 128)], wo.at[pl.ds(j * SK + r * n, n)], 0 if p1 else 1))
        nu = F // 64
        bounds = [(nu * j // WD_RC) * 64 for j in range(WD_RC + 1)]

        def slab(a, b, j, s):
            return cp(wd_hbm.at[pl.ds(a, b - a), pl.ds(j * 128, 128)], wd.at[pl.ds(j * F + a, b - a)], s)
        g_d01 = [slab(bounds[r], bounds[r + 1], j, 2) for r in range(WD_RC) for j in (0, 1)]
        g_d23 = [slab(bounds[r], bounds[r + 1], j, 0) for r in range(WD_RC) for j in (2, 3)]
        FS4 = opts.get('fs4', 10)
        if FS4 > 0:
            g_d4a = [slab(0, FS4 * 128, 4, 1)]
            g_d4b = [slab(FS4 * 128, F, 4, 2)]
        else:
            g_d4a = [slab(0, F, 4, 1)]
            g_d4b = []

        def start(grp):
            for c in grp:
                c.start()

        wcount = [0]

        def wait(grp):
            with scope('wait%02d' % wcount[0]):
                for c in grp:
                    c.wait()
            wcount[0] += 1

        start(g_q)
        start(g_uk)
        start(g_ckv)

        if opts.get('dmaonly', 0):
            wait(g_q); start(g_uv); wait(g_uk); start(g_g); wait(g_ckv); start(g_u); wait(g_uv); start(g_o1)
            wait(g_g); start(g_o2); wait(g_u); start(g_d01); wait(g_o1); start(g_d23); wait(g_o2); start(g_d4a); wait(g_d01); start(g_d4b); wait(g_d23); wait(g_d4a); wait(g_d4b)
            o_ref[...] = xb[...]
            return
        lane = _iota((8, 128), 1)
        sub = _iota((8, 128), 0)
        h16 = lane % 16
        XM = jnp.where(h16 == 2 * sub, np.uint32(0x0000FFFF),
                       jnp.where(h16 == 2 * sub + 1, np.uint32(0xFFFF0000), np.uint32(0)))
        idx16 = lane // 16
        PM = jnp.where(lane % 2 == 0, np.uint32(0x0000FFFF), np.uint32(0xFFFF0000))
        idx2 = lane // 2

        wq_u = wq.bitcast(U32)
        wuk_u = wuk.bitcast(U32)
        wuv_u = wuv.bitcast(U32)
        ckv_u = ckv.bitcast(U32)
        ckvT_u = ckvT.bitcast(U32)
        wo_u = wo.bitcast(U32)
        guT_u = guT.bitcast(U32)
        wd_u = wd.bitcast(U32)

        def xtile(w_u, g, hh):
            rows = [w_u[pl.ds((8 * g + j) * 16 + 8 * hh, 8), :] for j in range(8)]
            return pltpu.bitcast(jnp.concatenate(rows, axis=0), BF)

        def xlhs(src, r):
            return pltpu.bitcast(jnp.take_along_axis(src, idx16 + 8 * r, axis=1) & XM, BF)

        def xblock(srcs, w_u, blk, acc, hhs=(0, 1)):
            for r in range(16):
                l0 = None
                for hh in hhs:
                    if l0 is None or srcs[hh] is not srcs[hhs[0]]:
                        l0 = xlhs(srcs[hh], r)
                    acc[hh] = _acc(acc[hh], _dot(l0, xtile(w_u, 16 * blk + r, hh)))

        def dup_bits(v):
            u = pltpu.bitcast(v.astype(BF).astype(F32), U32)
            return u | (u >> 16)

        def colsum_q():
            if opts.get('no_cs', 0): return [jnp.zeros((16,128),F32)]*2
            l0 = pltpu.bitcast(XM & np.uint32(0x3F803F80), BF)
            acc = [None, None]
            for g in range(M // 8):
                for hh in range(2):
                    acc[hh] = _acc(acc[hh], _dot(l0, xtile(wq_u, g, hh)))
            return acc

        def relayout_uk():
            if opts.get('no_uk', 0): return
            for hp in range(16):
                for cb in range(NCB):
                    s = wuk_u[pl.ds(128 * cb * 16 + hp, 128, stride=16), :]
                    ukT[pl.ds((hp * NCB + cb) * 128, 128), :] = s.T

        def transpose_ckv():
            if opts.get('no_ckv', 0): return
            for cb in range(NCB):
                for kb in range(NKB):
                    t = ckv[pl.ds(cb * SK + kb * 128, 128), :]
                    ckvT[pl.ds((cb * NKB + kb) * 128, 128), :] = t.T

        def gu_index(which, fb, mb):
            return (which * NFB + fb) * NMB + mb

        def transpose_gu(which, src):
            if opts.get('no_gu', 0): return
            for fb in range(NFB):
                for mb in range(NMB):
                    t = src[pl.ds(fb * 128, 128), pl.ds(mb * 128, 128)]
                    guT[pl.ds(gu_index(which, fb, mb) * 128, 128), :] = t.T

        def transpose_gu_last():
            for mb in range(NMB):
                t = jnp.concatenate([wg[pl.ds(NFB * 128, FREM), pl.ds(mb * 128, 128)],
                                     wu[pl.ds(NFB * 128, FREM), pl.ds(mb * 128, 128)]], axis=0)
                guT[pl.ds((2 * NFB * NMB + mb) * 128, 128), :] = t.T

        def b_block(L, hh, cb):
            acc = None
            for hp8 in range(8):
                hp = hh * 8 + hp8
                for kh in range(2):
                    Lm = pltpu.bitcast(jnp.where(sub == hp8, L[kh], np.uint32(0)), BF)
                    acc = _acc(acc, _dot(Lm, _tile(ukT, (hp * NCB + cb) * 128 + 64 * kh)))
            return acc

        def b_lhs(qh):
            qp = _pack_rows(qh)
            return [jnp.take_along_axis(qp, idx2 + 64 * kh, axis=1) & PM for kh in range(2)]

        CEXP = (D ** -0.5) * LOG2E

        def sblk(kb):
            return s_scr.at[:, kb * 128:(kb + 1) * 128]

        def attention(q_raw, finish_q, csq, first):
            qa = [[None] * NCB for _ in range(2)]
            L0 = b_lhs(finish_q(q_raw[0], csq[0]))
            for cb in range(NCB):
                qa[0][cb] = b_block(L0, 0, cb)
            L1 = b_lhs(finish_q(q_raw[1], csq[1]))
            for cb in range(NCB - 1):
                qa[1][cb] = b_block(L1, 1, cb)

            def c_lhs(cb):
                return jnp.concatenate([qa[0][cb], qa[1][cb]], axis=0).astype(BF)
            if first:
                wait(g_ckv)
                start(g_u)
                transpose_ckv()
            lhs = [None] * NCB
            lhs[0] = c_lhs(0)
            for kb in range(NA):
                sblk(kb)[...] = _dot(lhs[0], _tile(ckvT_u, (0 * NKB + kb) * 64))
            qa[1][NCB - 1] = b_block(L1, 1, NCB - 1)
            mx = None
            for cb in range(1, NCB):
                lhs[cb] = c_lhs(cb)
                for kb in range(NA):
                    s = sblk(kb)[...] + _dot(lhs[cb], _tile(ckvT_u, (cb * NKB + kb) * 64))
                    sblk(kb)[...] = s
                    if cb == NCB - 1:
                        mx = s if mx is None else jnp.maximum(mx, s)
            mA = jnp.max(mx, axis=1, keepdims=True)
            for kb in range(NA, NKB):
                s = None
                for cb in range(NCB):
                    s = _acc(s, _dot(lhs[cb], _tile(ckvT_u, (cb * NKB + kb) * 64)))
                sblk(kb)[...] = s
                mx = jnp.maximum(mx, s)
            mB = jnp.max(mx, axis=1, keepdims=True)
            acc = [None] * NCB
            l = None
            for kb in range(NA):
                p = jnp.exp2((sblk(kb)[...] - mA) * CEXP)
                l = _acc(l, p)
                pb = p.astype(BF)
                for cb in range(NCB):
                    acc[cb] = _acc(acc[cb], _dot(pb, _tile(ckv_u, cb * (SK // 2) + kb * 64)))
            alpha = jnp.exp2((mA - mB) * CEXP)
            acc = [a * alpha for a in acc]
            l = l * alpha
            for kb in range(NA, NKB - NB2):
                p = jnp.exp2((sblk(kb)[...] - mB) * CEXP)
                l = l + p
                pb = p.astype(BF)
                for cb in range(NCB):
                    acc[cb] = acc[cb] + _dot(pb, _tile(ckv_u, cb * (SK // 2) + kb * 64))
            pbs = []
            for kb in range(NKB - NB2, NKB):
                p = jnp.exp2((sblk(kb)[...] - mB) * CEXP)
                l = l + p
                pbs.append(p.astype(BF))
            linv = 1.0 / jnp.sum(l, axis=1, keepdims=True)
            srcs = []
            for cb in range(NCB):
                for i, kb in enumerate(range(NKB - NB2, NKB)):
                    acc[cb] = acc[cb] + _dot(pbs[i], _tile(ckv_u, cb * (SK // 2) + kb * 64))
                cc = acc[cb] * linv
                srcs.append([_pack_rows(cc[0:16]), _pack_rows(cc[16:32])])
            if first:
                wait(g_uv)
                start(g_o1)
            ctx = [None, None]
            for cb in range(NCB - 1):
                xblock(srcs[cb], wuv_u, cb, ctx)
            xblock(srcs[NCB - 1], wuv_u, NCB - 1, ctx, hhs=(0,))
            xblock(srcs[NCB - 1], wuv_u, NCB - 1, ctx, hhs=(1,))
            return ctx

        def paced(mxu_fns, vpu_fns, depd, rho_scale=1.0):
            rho = len(vpu_fns) / max(1, len(mxu_fns)) * rho_scale
            res = []
            j = 0
            for t, fn in enumerate(mxu_fns):
                res.append(fn())
                while j < len(vpu_fns) and j < rho * (t + 1):
                    vpu_fns[j](res[max(t - depd, 0)] if depd >= 0 else None)
                    j += 1
            while j < len(vpu_fns):
                vpu_fns[j](None)
                j += 1

        def tie(v, dep):
            if dep is None:
                return v
            return jnp.where(always, v, pltpu.bitcast(dep, U32))

        def silu(g):
            return g / (1.0 + jnp.exp(-g))

        ones8 = jnp.ones((8, 128), F32)

        def mix(x, ctx, first):
            if first:
                wait(g_g)
                start(g_o2)
                transpose_gu(0, wg)
                wait(g_u)
                start(g_d01)
                transpose_gu(1, wu)
                transpose_gu_last()
                onesL = jnp.ones((16, 128), BF)
                for i, fb in enumerate(tuple(opts.get('gv', ()))):
                    for which in range(2):
                        a = None
                        for mb in range(NMB):
                            a = _acc(a, _dot(onesL, _tile(guT_u, gu_index(which, fb, mb) * 64))[0:8])
                        cs_scr[pl.ds((2 * i + which) * 8, 8), :] = a
                wait(g_o1)
                start(g_d23)
            def flhs(h):
                hh, r = divmod(h, 16)
                return jnp.broadcast_to(ctx[hh][r:r + 1, :], (16, 128)).astype(BF)
            FV = opts.get('fv', ())
            acc = [None] * NMB
            vlo = [None] * NMB
            vhi = [None] * NMB

            mts = {}

            def f_group(h, k, dep):
                if h not in mts:
                    L = flhs(h)
                    mts[h] = pltpu.bitcast(jnp.concatenate([L] * 8, axis=0).T, U32)
                mk = mts[h][8 * k:8 * k + 8]
                if dep is not None:
                    mk = jnp.where(always, mk, pltpu.bitcast(dep, U32))
                mlo, mhi = unpack(mk)
                for mb in range(NMB):
                    wlo, whi = unpack(wo_u[pl.ds(mb * (SK // 2) + h * 64 + 8 * k, 8), :])
                    vlo[mb] = _acc(vlo[mb], wlo * mlo + whi * mhi)

            DEPD = opts.get('depd', 2)
            RHO = opts.get('rho', 1.0)

            def run_mixed(mh, vh, mb_major):
                groups = [(h, k) for h in vh for k in range(8)]
                tiles = [(h, mb) for mb in range(NMB) for h in mh] if mb_major else [(h, mb) for h in mh for mb in range(NMB)]
                rho = len(groups) / max(1, len(tiles)) * RHO
                res = []
                j = 0
                Lc = {}
                for t, (h, mb) in enumerate(tiles):
                    if h not in Lc:
                        Lc[h] = flhs(h)
                    acc[mb] = _acc(acc[mb], _dot(Lc[h], _tile(wo_u, mb * (SK // 2) + h * 64))[0:8])
                    res.append(acc[mb])
                    while j < len(groups) and j < rho * (t + 1):
                        f_group(*groups[j], res[t - DEPD] if (t >= DEPD and DEPD >= 0) else None)
                        j += 1
                while j < len(groups):
                    f_group(*groups[j], None)
                    j += 1
            run_mixed([h for h in range(NH1) if h not in FV], [h for h in range(NH1) if h in FV], False)
            if first:
                wait(g_o2)
                start(g_d4a)
            assert all(h < NH1 for h in FV)
            Ls = {h: flhs(h) for h in range(NH1, 32) if h not in FV}
            x1 = []
            for mb in range(NMB):
                for h in Ls:
                    acc[mb] = _acc(acc[mb], _dot(Ls[h], _tile(wo_u, mb * (SK // 2) + h * 64))[0:8])
                a = acc[mb]
                if FV:
                    a = a + jnp.sum(vlo[mb], axis=0, keepdims=True)
                x1.append(x[mb] + a)
            GV = tuple(opts.get('gv', ()))
            L = [jnp.concatenate([x1[b], ones8], axis=0).astype(BF) for b in range(NMB)]
            mean, inv = _stats(x1)
            xn1 = [(x1[b] - mean) * inv for b in range(NMB)]
            rr = xn1[0] * wr_rows[0]
            for b in range(1, NMB):
                rr = rr + xn1[b] * wr_rows[b]
            r = jnp.sum(rr, axis=1, keepdims=True)
            sig = 1.0 / (1.0 + jnp.exp(-r))

            def fin(a):
                return (a[0:8] - mean * a[8:16]) * inv
            hs = [None] * NFB
            accs = {}
            mfb = [fb for fb in range(NFB) if fb not in GV]
            mxu_fns = []

            HV = tuple(opts.get('hv', ()))
            mth = {}

            def g_tile(fb, which, mb):
                def fn():
                    accs[fb, which] = _acc(accs.get((fb, which)), _dot(L[mb], _tile(guT_u, gu_index(which, fb, mb) * 64)))
                    res = accs[fb, which][0:8]
                    if which == 1 and mb == NMB - 1 and opts.get('early_hs', 1):
                        hs[fb] = silu(fin(accs[fb, 0])) * fin(accs[fb, 1])
                        if fb in HV and not first:
                            mth[fb] = pltpu.bitcast(jnp.concatenate([_rep16(hs[fb])] * 8, axis=0).T, U32)
                    return res
                return fn
            for mb in range(NMB):
                for fb in mfb[:G1]:
                    for which in range(2):
                        mxu_fns.append(g_tile(fb, which, mb))
            for fb in mfb[G1:]:
                for which in range(2):
                    for mb in range(NMB):
                        mxu_fns.append(g_tile(fb, which, mb))
            vacc = {}
            mtg = {}

            def g_group(mb, k, which):
                def fn(dep):
                    if mb not in mtg:
                        mtg[mb] = pltpu.bitcast(jnp.concatenate([_rep16(x1[mb])] * 8, axis=0).T, U32)
                    mlo, mhi = unpack(tie(mtg[mb][8 * k:8 * k + 8], dep))
                    for fb in GV:
                        wlo, whi = unpack(guT_u[pl.ds(gu_index(which, fb, mb) * 64 + 8 * k, 8), :])
                        vacc[fb, which] = _acc(vacc.get((fb, which)), wlo * mlo + whi * mhi)
                return fn
            vpu_fns = [g_group(mb, k, which) for mb in range(NMB) for k in range(8) for which in range(2)] if GV else []
            paced(mxu_fns, vpu_fns, opts.get('gdepd', 2), opts.get('grho', 1.0))
            for fb in mfb:
                if hs[fb] is None:
                    hs[fb] = silu(fin(accs[fb, 0])) * fin(accs[fb, 1])
            for i, fb in enumerate(GV):
                gu = []
                for which in range(2):
                    raw = jnp.sum(vacc[fb, which], axis=0, keepdims=True)
                    gu.append((raw - mean * cs_scr[pl.ds((2 * i + which) * 8, 8), :]) * inv)
                hs[fb] = silu(gu[0]) * gu[1]
            a = None
            for mb in range(NMB):
                a = _acc(a, _dot(L[mb], _tile(guT_u, (2 * NFB * NMB + mb) * 64)))
            a = fin(a)
            sw = pltpu.roll(a, 64, axis=1)
            g = jnp.where(lane < 64, a, sw)
            u = jnp.where(lane < 64, sw, a)
            hs.append(silu(g) * u)
            return x1, xn1, sig, hs, mth

        def h_last_lhs(hl):
            z = jnp.zeros_like(hl)
            ev = jnp.where(lane < 64, hl, z)
            od = jnp.where(lane < 64, z, hl)
            return _rep16(jnp.where(sub % 2 == 0, ev, od))

        def h_last_tile(L, mb, mb2):
            r0 = NFB * 64
            t = jnp.concatenate([wd_u[pl.ds(mb * (F // 2) + r0, 32), :], wd_u[pl.ds(mb2 * (F // 2) + r0, 32), :]], axis=0)
            return _dot(L, pltpu.bitcast(t, BF))[0:8]

        def h_fb_major(hs, mth):
            GV = tuple(opts.get('gv', ()))
            HV = tuple(opts.get('hv', ()))
            acc = [None] * NMB
            order = [fb for fb in range(NFB) if fb not in GV] + [NFB] + list(GV)
            mxu_fns = []
            Lc = {}

            def h_tile(fb, mb):
                def fn():
                    if fb not in Lc:
                        Lc[fb] = _rep16(hs[fb])
                    acc[mb] = _acc(acc[mb], _dot(Lc[fb], _tile(wd_u, mb * (F // 2) + fb * 64))[0:8])
                    return acc[mb]
                return fn

            def h_last(mb):
                def fn():
                    if NFB not in Lc:
                        Lc[NFB] = h_last_lhs(hs[NFB])
                    mb2 = min(mb + 1, NMB - 1)
                    o = h_last_tile(Lc[NFB], mb, mb2)
                    acc[mb] = acc[mb] + jnp.broadcast_to(o[0:1], (8, 128))
                    if mb2 != mb:
                        acc[mb2] = acc[mb2] + jnp.broadcast_to(o[1:2], (8, 128))
                    return acc[mb]
                return fn
            for fb in order:
                if fb in HV:
                    continue
                if fb == NFB:
                    mxu_fns += [h_last(mb) for mb in range(0, NMB, 2)]
                else:
                    mxu_fns += [h_tile(fb, mb) for mb in range(NMB)]
            vacc = [None] * NMB

            def h_group(fb, k):
                def fn(dep):
                    if fb not in mth:
                        mth[fb] = pltpu.bitcast(jnp.concatenate([_rep16(hs[fb])] * 8, axis=0).T, U32)
                    mlo, mhi = unpack(tie(mth[fb][8 * k:8 * k + 8], dep))
                    for mb in range(NMB):
                        wlo, whi = unpack(wd_u[pl.ds(mb * (F // 2) + fb * 64 + 8 * k, 8), :])
                        vacc[mb] = _acc(vacc[mb], wlo * mlo + whi * mhi)
                return fn
            paced(mxu_fns, [h_group(fb, k) for fb in HV for k in range(8)], opts.get('hdepd', 2), opts.get('hrho', 1.0))
            if HV:
                acc = [acc[mb] + jnp.sum(vacc[mb], axis=0, keepdims=True) for mb in range(NMB)]
            return acc

        def next_layer_head(x1, xn1, sig, hs, first):
            Lh = [_rep16(hs[fb]) for fb in range(NFB)]
            Ll = h_last_lhs(hs[NFB])
            acc = [None] * NMB
            x2 = [None] * NMB
            q = [None, None]

            def hpart(fbs, mbs):
                for fb in fbs:
                    for mb in mbs:
                        acc[mb] = _acc(acc[mb], _dot(Lh[fb], _tile(wd_u, mb * (F // 2) + fb * 64))[0:8])

            def hlast(mb, mb2):
                o = h_last_tile(Ll, mb, mb2)
                acc[mb] = acc[mb] + jnp.broadcast_to(o[0:1], (8, 128))
                if mb2 != mb:
                    acc[mb2] = acc[mb2] + jnp.broadcast_to(o[1:2], (8, 128))

            NDEF = opts.get('ndef', 8)
            ds = {}

            def finish_x(mb):
                x2[mb] = x1[mb] + xn1[mb] + acc[mb] * sig
                ds[mb] = dup_bits(x2[mb])

            def ablock(mb, rs, hhs=(0, 1)):
                for r in rs:
                    l0 = xlhs(ds[mb], r)
                    for hh in hhs:
                        q[hh] = _acc(q[hh], _dot(l0, xtile(wq_u, 16 * mb + r, hh)))

            if first:
                wait(g_d01)
                start(g_d4b)
            hpart(range(NFB), (0, 1))
            hlast(0, 1)
            finish_x(0)
            finish_x(1)
            ablock(0, range(16))
            ablock(1, range(16))
            if first:
                wait(g_d23)
            hpart(range(NFB), (2,))
            hlast(2, 2)
            hpart(range(NFB), (3,))
            hlast(3, 3)
            finish_x(2)
            finish_x(3)
            ablock(2, range(16))
            ablock(3, range(16 - NDEF))
            mb = NMB - 1
            if first:
                wait(g_d4a)
            hpart(range(FS4), (mb,))
            if first and g_d4b:
                wait(g_d4b)
            if first and opts.get('stop', 0):
                return x2[:4] + [acc[mb]], q
            hpart(range(FS4, NFB), (mb,))
            hlast(mb, mb)
            ablock(3, range(16 - NDEF, 16))
            finish_x(mb)
            ablock(mb, range(16), hhs=(0,))
            ablock(mb, range(16), hhs=(1,))
            return x2, q

        wait(g_q)
        start(g_uv)
        xrow = xb[0].astype(F32)
        x = [jnp.broadcast_to(xrow[:, b * 128:(b + 1) * 128], (8, 128)) for b in range(NMB)]
        wrf = wrb[...].astype(F32)
        wr_rows = [jnp.broadcast_to(wrf[b:b + 1, :], (8, 128)) for b in range(NMB)]
        always = (pltpu.bitcast(wr_rows[0], U32) | np.uint32(1)) != np.uint32(0)
        csq = colsum_q()
        q = [None, None]
        for mb in range(NMB):
            d = dup_bits(x[mb])
            xblock([d, d], wq_u, mb, q)

        def make_finish(x):
            mean, inv = _stats(x)
            return lambda raw, cs: (raw - mean[0:1] * cs) * inv[0:1]
        wait(g_uk)
        start(g_g)
        relayout_uk()
        ctx = attention(q, make_finish(x), csq, True)
        x1, xn1, sig, hs, mth = mix(x, ctx, True)
        for it in range(1 + extra):
            x, q = next_layer_head(x1, xn1, sig, hs, it == 0)
            if opts.get('stop', 0):
                out = jnp.concatenate([xb_[0:1] + q[0][0:1] + q[1][0:1] for xb_ in x], axis=1)
                o_ref[...] = out.astype(BF).reshape(1, 1, M)
                return
            with contextlib.nullcontext():
                ctx = attention(q, make_finish(x), csq, False)
            with contextlib.nullcontext():
                x1, xn1, sig, hs, mth = mix(x, ctx, False)
        with contextlib.nullcontext():
            acc = h_fb_major(hs, mth)
        xo = [x1[b] + xn1[b] + acc[b] * sig for b in range(NMB)]
        out = jnp.concatenate([xb_[0:1] for xb_ in xo], axis=1)
        o_ref[...] = out.astype(BF).reshape(1, 1, M)

    scratch = [
        pltpu.VMEM((1, 1, M), BF),
        pltpu.VMEM((NMB, 128), BF),
        pltpu.VMEM((M * H, D), BF),
        pltpu.VMEM((DC * H, D), BF),
        pltpu.VMEM((DC * H // 2, D), U32),
        pltpu.VMEM((NCB * SK, 128), BF),
        pltpu.VMEM((NCB * SK, 128), BF),
        pltpu.VMEM((DC * H, D), BF),
        pltpu.VMEM((NMB * SK, 128), BF),
        pltpu.VMEM((F, M), BF),
        pltpu.VMEM((F, M), BF),
        pltpu.VMEM(((2 * NFB * NMB + NMB) * 128, 128), BF),
        pltpu.VMEM((NMB * F, 128), BF),
        pltpu.VMEM((H, SK), F32),
        pltpu.VMEM((2 * NFB * 8, 128), F32),
        pltpu.SemaphoreType.DMA((3,)),
    ]

    def fn(A_x, A_c_kv, A_w_q, A_w_uk, A_w_uv, A_w_o, B_x, B_w_r, B_w_gate, B_w_up, B_w_down):
        return pl.pallas_call(
            kernel,
            out_shape=jax.ShapeDtypeStruct((1, 1, M), BF),
            in_specs=[pl.BlockSpec(memory_space=pltpu.HBM)] * 10,
            out_specs=pl.BlockSpec(memory_space=pltpu.VMEM),
            scratch_shapes=scratch,
            compiler_params=pltpu.CompilerParams(vmem_limit_bytes=100 * 1024 * 1024, flags=opts.get('flags', None)),
        )(A_x, B_w_r.reshape(NMB, 128), A_w_q.reshape(M * H, D), A_w_uk.reshape(DC * H, D),
          A_c_kv.reshape(SK, DC), A_w_uv.reshape(DC * H, D), A_w_o.reshape(H * D, M),
          B_w_gate.T, B_w_up.T, B_w_down)
    return fn


@jax.jit
def pallas_interleave_layers__compressed_kv_cla__moe_arch_mod__decode_kernel(
    A_x: jax.Array,
    A_c_kv: jax.Array,
    A_w_q: jax.Array,
    A_w_uk: jax.Array,
    A_w_uv: jax.Array,
    A_w_o: jax.Array,
    B_x: jax.Array,
    B_w_r: jax.Array,
    B_w_gate: jax.Array,
    B_w_up: jax.Array,
    B_w_down: jax.Array,
):
    fn = build({'ndef':16,'fs4':0,'nh1':28,'fv':(1,3,5,7,9,11,13,15,17,19),'gv':(9,10,11,12),'hv':(0,1,2,3),'depd':1,'grho':0.9})
    return fn(A_x, A_c_kv, A_w_q, A_w_uk, A_w_uv, A_w_o, B_x, B_w_r, B_w_gate, B_w_up, B_w_down)
```

```python
import functools
import contextlib
import numpy as np
import jax
import jax.numpy as jnp
from jax import lax
import jax.experimental.pallas as pl
import jax.experimental.pallas.tpu as pltpu

M, H, D, DC, SK, F = 640, 32, 128, 512, 4096, 1728
NMB = M // 128
NCB = DC // 128
NKB = SK // 128
NFB = F // 128
FREM = F - NFB * 128
LOG2E = 1.4426950408889634
EPS = 1e-5
BF = jnp.bfloat16
F32 = jnp.float32
U32 = jnp.uint32


def _dot(a, b):
    return jnp.dot(a, b, preferred_element_type=F32)


def _tile(ref_u32, r0):
    return pltpu.bitcast(ref_u32[pl.ds(r0, 64), :], BF)


def _iota(shape, ax):
    return lax.broadcasted_iota(jnp.int32, shape, ax)


def _pack_rows(v):
    return pltpu.bitcast(v.astype(BF), U32)


def _stats(x):
    s = x[0]
    for b in range(1, NMB):
        s = s + x[b]
    mean = jnp.sum(s, axis=1, keepdims=True) * (1.0 / M)
    xc = [xb - mean for xb in x]
    v = xc[0] * xc[0]
    for b in range(1, NMB):
        v = v + xc[b] * xc[b]
    var = jnp.sum(v, axis=1, keepdims=True) * (1.0 / M)
    return mean, lax.rsqrt(var + EPS)


def _stats_shift(x, shift):
    d = [xb - shift for xb in x]
    s1 = d[0]
    s2 = d[0] * d[0]
    for b in range(1, NMB):
        s1 = s1 + d[b]
        s2 = s2 + d[b] * d[b]
    m1 = jnp.sum(s1, axis=1, keepdims=True) * (1.0 / M)
    m2 = jnp.sum(s2, axis=1, keepdims=True) * (1.0 / M)
    var = jnp.maximum(m2 - m1 * m1, 0.0)
    return shift + m1, lax.rsqrt(var + EPS)


def _rep16(v):
    return jnp.concatenate([v, v], axis=0).astype(BF)


def unpack(w):
    lo = pltpu.bitcast(w << 16, F32)
    hi = pltpu.bitcast(w & np.uint32(0xFFFF0000), F32)
    return lo, hi


def _acc(a, o):
    return o if a is None else a + o


def build(opts=None):
    opts = dict(opts or {})
    WO_RC = opts.get('wo_rc', 8)
    WD_RC = opts.get('wd_rc', 12)
    WD_SPLIT = opts.get('wd_split', 9)
    NA = opts.get('na', 8)
    NB2 = opts.get('nb2', 8)
    G1 = opts.get('g1', 3)
    scoped = opts.get('scoped', False)
    extra = opts.get('extra', 0)

    def scope(name):
        if scoped:
            return jax.named_scope(name)
        import contextlib
        return contextlib.nullcontext()

    def kernel(x_hbm, wr_hbm, wq_hbm, wuk_hbm, ckv_hbm, wuv_hbm, wo_hbm, wg_hbm, wu_hbm, wd_hbm,
               o_ref,
               xb, wrb, wq, wuk, ukT, ckv, ckvT, wuv, wo, wg, wu, guT, wd, s_scr, cs_scr, mt_scr, sems):
        def cp(src, dst, s):
            return pltpu.make_async_copy(src, dst, sems.at[s])
        g_q = [cp(wq_hbm, wq, 0), cp(x_hbm, xb, 0), cp(wr_hbm, wrb, 0)]
        g_uk = [cp(wuk_hbm, wuk, 1)]
        g_ckv = [cp(ckv_hbm.at[:, pl.ds(j * 128, 128)], ckv.at[pl.ds(j * SK, SK)], 2) for j in range(NCB)]
        g_uv = [cp(wuv_hbm, wuv, 0)]
        g_g = [cp(wg_hbm, wg, 1)]
        g_u = [cp(wu_hbm, wu, 2)]
        NH1 = opts.get('nh1', 24)
        g_o1, g_o2 = [], []
        for r in range(WO_RC):
            n = SK // WO_RC
            for j in range(NMB):
                p1 = r * n < NH1 * D
                (g_o1 if p1 else g_o2).append(
                    cp(wo_hbm.at[pl.ds(r * n, n), pl.ds(j * 128, 128)], wo.at[pl.ds(j * SK + r * n, n)], 0 if p1 else 1))
        nu = F // 64
        bounds = [(nu * j // WD_RC) * 64 for j in range(WD_RC + 1)]

        def slab(a, b, j, s):
            return cp(wd_hbm.at[pl.ds(a, b - a), pl.ds(j * 128, 128)], wd.at[pl.ds(j * F + a, b - a)], s)
        g_d01 = [slab(bounds[r], bounds[r + 1], j, 2) for r in range(WD_RC) for j in (0, 1)]
        RS = opts.get('rs23', 9)
        FS23 = bounds[RS] // 128
        g_d23a = [slab(bounds[r], bounds[r + 1], j, 0) for r in range(RS) for j in (2, 3)]
        g_d23b = [slab(bounds[r], bounds[r + 1], j, 1) for r in range(RS, WD_RC) for j in (2, 3)]
        FS4 = opts.get('fs4', 10)
        assert FS4 == 0
        g_d4a = [slab(0, F, 4, 2)]
        g_d4b = []

        def start(grp):
            for c in grp:
                c.start()

        wcount = [0]

        def wait(grp):
            with scope('wait%02d' % wcount[0]):
                for c in grp:
                    c.wait()
            wcount[0] += 1

        start(g_q)
        start(g_uk)
        start(g_ckv)

        if opts.get('dmaonly', 0):
            wait(g_q); start(g_uv); wait(g_uk); start(g_g); wait(g_ckv); start(g_u); wait(g_uv); start(g_o1)
            wait(g_g); start(g_o2); wait(g_u); start(g_d01); wait(g_o1); start(g_d23a); wait(g_o2); start(g_d23b); wait(g_d01); start(g_d4a); wait(g_d23a); wait(g_d23b); wait(g_d4a)
            o_ref[...] = xb[...]
            return
        lane = _iota((8, 128), 1)
        sub = _iota((8, 128), 0)
        h16 = lane % 16
        XM = jnp.where(h16 == 2 * sub, np.uint32(0x0000FFFF),
                       jnp.where(h16 == 2 * sub + 1, np.uint32(0xFFFF0000), np.uint32(0)))
        rlo, rhi = 2 * sub, 2 * sub + 1
        hlo = jnp.where(rlo < 8, 2 * rlo, 2 * (rlo - 8) + 1)
        hhi = jnp.where(rhi < 8, 2 * rhi, 2 * (rhi - 8) + 1)
        XQ = (jnp.where(h16 == hlo, np.uint32(0x0000FFFF), np.uint32(0))
              | jnp.where(h16 == hhi, np.uint32(0xFFFF0000), np.uint32(0)))
        idx16 = lane // 16
        PM = jnp.where(lane % 2 == 0, np.uint32(0x0000FFFF), np.uint32(0xFFFF0000))
        idx2 = lane // 2

        wq_u = wq.bitcast(U32)
        wuk_u = wuk.bitcast(U32)
        wuv_u = wuv.bitcast(U32)
        mt_u = mt_scr.bitcast(U32)
        ukT_u = ukT.bitcast(U32)
        ckv_u = ckv.bitcast(U32)
        ckvT_u = ckvT.bitcast(U32)
        wo_u = wo.bitcast(U32)
        guT_u = guT.bitcast(U32)
        wd_u = wd.bitcast(U32)

        def xtile(w_u, g, hh):
            rows = [w_u[pl.ds((8 * g + j) * 16 + 8 * hh, 8), :] for j in range(8)]
            return pltpu.bitcast(jnp.concatenate(rows, axis=0), BF)

        def xlhs(src, r, mask=None):
            mask = XM if mask is None else mask
            return pltpu.bitcast(jnp.take_along_axis(src, idx16 + 8 * r, axis=1) & mask, BF)

        def xblock(srcs, w_u, blk, acc, hhs=(0, 1), mask=None):
            for r in range(16):
                l0 = None
                for hh in hhs:
                    if l0 is None or srcs[hh] is not srcs[hhs[0]]:
                        l0 = xlhs(srcs[hh], r, mask)
                    acc[hh] = _acc(acc[hh], _dot(l0, xtile(w_u, 16 * blk + r, hh)))

        def dup_bits(v):
            u = pltpu.bitcast(v.astype(BF).astype(F32), U32)
            return u | (u >> 16)

        def colsum_q():
            if opts.get('no_cs', 0): return [jnp.zeros((16,128),F32)]*2
            l0 = pltpu.bitcast(XQ & np.uint32(0x3F803F80), BF)
            acc = [None, None]
            for g in range(M // 8):
                for hh in range(2):
                    acc[hh] = _acc(acc[hh], _dot(l0, xtile(wq_u, g, hh)))
            return acc

        def relayout_uk():
            if opts.get('no_uk', 0): return
            for hp in range(16):
                for cb in range(NCB):
                    s = wuk_u[pl.ds(128 * cb * 16 + hp, 128, stride=16), :]
                    ukT[pl.ds((hp * NCB + cb) * 256, 256), :] = pltpu.bitcast(s.T, BF)

        def transpose_ckv():
            if opts.get('no_ckv', 0): return
            for cb in range(NCB):
                for kb in range(NKB):
                    t = ckv[pl.ds(cb * SK + kb * 128, 128), :]
                    ckvT[pl.ds((cb * NKB + kb) * 128, 128), :] = t.T

        def gu_index(which, fb, mb):
            return (which * NFB + fb) * NMB + mb

        def transpose_gu(which, src):
            if opts.get('no_gu', 0): return
            for fb in range(NFB):
                for mb in range(NMB):
                    t = src[pl.ds(fb * 128, 128), pl.ds(mb * 128, 128)]
                    guT[pl.ds(gu_index(which, fb, mb) * 128, 128), :] = t.T

        def transpose_gu_last():
            for mb in range(NMB):
                t = jnp.concatenate([wg[pl.ds(NFB * 128, FREM), pl.ds(mb * 128, 128)],
                                     wu[pl.ds(NFB * 128, FREM), pl.ds(mb * 128, 128)]], axis=0)
                guT[pl.ds((2 * NFB * NMB + mb) * 128, 128), :] = t.T

        def b_block(L, hh, cb):
            acc = None
            for hp8 in range(8):
                hp = hh * 8 + hp8
                for kh in range(2):
                    Lm = pltpu.bitcast(jnp.where(sub == hp8, L[kh], np.uint32(0)), BF)
                    acc = _acc(acc, _dot(Lm, _tile(ukT_u, (hp * NCB + cb) * 128 + 64 * kh)))
            return acc

        def b_lhs(qh):
            qp = _pack_rows(qh)
            return [jnp.take_along_axis(qp, idx2 + 64 * kh, axis=1) & PM for kh in range(2)]

        CEXP = (D ** -0.5) * LOG2E

        def sblk(kb):
            return s_scr.at[:, kb * 128:(kb + 1) * 128]

        def attention(q_raw, finish_q, csq, first, pre_fns=(), pre_v=()):
            BV = tuple(opts.get('bv', ()))
            qa = [[None] * NCB for _ in range(2)]
            qps = {}

            def get_qp(hh):
                if hh not in qps:
                    qf = finish_q(q_raw[hh], csq[hh], hh)
                    qps[hh] = pltpu.bitcast(pltpu.pack_elementwise([qf[0:8], qf[8:16]], packed_dtype=BF), U32)
                return qps[hh]
            Lb = {}

            def b_tile(hh, cb, hp8, kh):
                def fn():
                    if hh not in Lb:
                        qp = get_qp(hh)
                        Lb[hh] = [jnp.take_along_axis(qp, idx2 + 64 * k2, axis=1) & PM for k2 in range(2)]
                    Lm = pltpu.bitcast(jnp.where(sub == hp8, Lb[hh][kh], np.uint32(0)), BF)
                    o = _dot(Lm, _tile(ukT_u, ((hh * 8 + hp8) * NCB + cb) * 128 + 64 * kh))
                    qa[hh][cb] = _acc(qa[hh][cb], o)
                    return o[0:8]
                return fn

            def b_fns(hh, cb):
                return [b_tile(hh, cb, hp8, kh) for hp8 in range(8) if (hh * 8 + hp8) not in BV for kh in range(2)]
            mtb = {}
            blo, bhi = {}, {}

            def mk_mtb(hp):
                if hp not in mtb:
                    qp = get_qp(hp // 8)
                    mtb[hp] = jnp.broadcast_to(qp[hp % 8:hp % 8 + 1, :], (128, 128)).T

            def b_group(hp, k):
                def fn(dep):
                    mk_mtb(hp)
                    i = BV.index(hp)
                    for ahead in range(1, opts.get('bahead', 0) + 1):
                        if i + ahead < len(BV):
                            mk_mtb(BV[i + ahead])
                    mlo, mhi = unpack(tie(mtb[hp][8 * k:8 * k + 8], dep))
                    for cb in range(NCB):
                        wlo, whi = unpack(ukT_u[pl.ds((hp * NCB + cb) * 128 + 8 * k, 8), :])
                        blo[hp, cb] = _acc(blo.get((hp, cb)), wlo * mlo)
                        bhi[hp, cb] = _acc(bhi.get((hp, cb)), whi * mhi)
                    return blo[hp, NCB - 1]
                return fn
            if BV:
                mk_mtb(BV[0])
                if len(BV) > 1 and opts.get('bahead', 0):
                    mk_mtb(BV[1])
            mfns = list(pre_fns)
            for cb in range(NCB):
                mfns += b_fns(0, cb)
            for cb in range(NCB - 1):
                mfns += b_fns(1, cb)
            paced(mfns, list(pre_v) + [b_group(hp, k) for hp in BV for k in range(16)], opts.get('bdepd', 2), opts.get('brho', 1.0), opts.get('bskip', 0))
            for hp in BV:
                hh, hp8 = divmod(hp, 8)
                v, r0 = hp8 // 4, 2 * (hp8 % 4)
                for cb in range(NCB):
                    lo, hi = blo[hp, cb], bhi[hp, cb]
                    u = jnp.where(sub % 2 == 0, lo + pltpu.roll(lo, 7, axis=0), hi + pltpu.roll(hi, 1, axis=0))
                    u = u + pltpu.roll(u, 2, axis=0)
                    u = u + pltpu.roll(u, 4, axis=0)
                    parts = [qa[hh][cb][0:8], qa[hh][cb][8:16]]
                    parts[v] = jnp.where((sub == r0) | (sub == r0 + 1), u, parts[v])
                    qa[hh][cb] = jnp.concatenate(parts, axis=0)

            def c_lhs(cb):
                return jnp.concatenate([qa[0][cb], qa[1][cb]], axis=0).astype(BF)
            if first:
                wait(g_ckv)
                start(g_u)
                transpose_ckv()
            lhs = [None] * NCB
            lhs[0] = c_lhs(0)
            for kb in range(NA):
                sblk(kb)[...] = _dot(lhs[0], _tile(ckvT_u, (0 * NKB + kb) * 64))
            for fn in b_fns(1, NCB - 1):
                fn()
            mx = None
            for cb in range(1, NCB):
                lhs[cb] = c_lhs(cb)
                for kb in range(NA):
                    s = sblk(kb)[...] + _dot(lhs[cb], _tile(ckvT_u, (cb * NKB + kb) * 64))
                    sblk(kb)[...] = s
                    if cb == NCB - 1:
                        mx = s if mx is None else jnp.maximum(mx, s)
            mA = jnp.max(mx, axis=1, keepdims=True)
            for kb in range(NA, NKB):
                s = None
                for cb in range(NCB):
                    s = _acc(s, _dot(lhs[cb], _tile(ckvT_u, (cb * NKB + kb) * 64)))
                sblk(kb)[...] = s
                mx = jnp.maximum(mx, s)
            mB = jnp.max(mx, axis=1, keepdims=True)
            acc = [None] * NCB
            l = None
            for kb in range(NA):
                p = jnp.exp2((sblk(kb)[...] - mA) * CEXP)
                l = _acc(l, p)
                pb = p.astype(BF)
                for cb in range(NCB):
                    acc[cb] = _acc(acc[cb], _dot(pb, _tile(ckv_u, cb * (SK // 2) + kb * 64)))
            alpha = jnp.exp2((mA - mB) * CEXP)
            acc = [a * alpha for a in acc]
            l = l * alpha
            for kb in range(NA, NKB - NB2):
                p = jnp.exp2((sblk(kb)[...] - mB) * CEXP)
                l = l + p
                pb = p.astype(BF)
                for cb in range(NCB):
                    acc[cb] = acc[cb] + _dot(pb, _tile(ckv_u, cb * (SK // 2) + kb * 64))
            pbs = []
            for kb in range(NKB - NB2, NKB):
                p = jnp.exp2((sblk(kb)[...] - mB) * CEXP)
                l = l + p
                pbs.append(p.astype(BF))
            linv = 1.0 / jnp.sum(l, axis=1, keepdims=True)
            srcs = []
            for cb in range(NCB):
                for i, kb in enumerate(range(NKB - NB2, NKB)):
                    acc[cb] = acc[cb] + _dot(pbs[i], _tile(ckv_u, cb * (SK // 2) + kb * 64))
                cc = acc[cb] * linv
                srcs.append([_pack_rows(cc[0:16]), _pack_rows(cc[16:32])])
            if first:
                wait(g_uv)
                start(g_o1)
            ctx = [None, None]
            for cb in range(NCB - 1):
                xblock(srcs[cb], wuv_u, cb, ctx)
            xblock(srcs[NCB - 1], wuv_u, NCB - 1, ctx, hhs=(0,))
            xblock(srcs[NCB - 1], wuv_u, NCB - 1, ctx, hhs=(1,))
            return ctx

        def paced(mxu_fns, vpu_fns, depd, rho_scale=1.0, skip=0):
            rho = len(vpu_fns) / max(1, len(mxu_fns) - skip) * rho_scale
            SELF = opts.get('self', 0)
            res = []
            vres = []
            j = 0

            def run_v(t):
                if SELF:
                    dep = vres[j - SELF] if j >= SELF else None
                else:
                    dep = res[max(t - depd, 0)] if depd >= 0 else None
                vres.append(vpu_fns[j](dep))
            for t, fn in enumerate(mxu_fns):
                res.append(fn())
                while j < len(vpu_fns) and j < rho * (t + 1 - skip):
                    run_v(t)
                    j += 1
            while j < len(vpu_fns):
                run_v(len(mxu_fns) - 1)
                j += 1

        def tie(v, dep):
            if dep is None:
                return v
            return jnp.where(always, v, pltpu.bitcast(dep, U32))

        def silu(g):
            return g / (1.0 + jnp.exp(-g))

        ones8 = jnp.ones((8, 128), F32)

        def mix(x, ctx, first, fuse_h=False):
            if first:
                wait(g_g)
                start(g_o2)
                transpose_gu(0, wg)
                wait(g_u)
                start(g_d01)
                transpose_gu(1, wu)
                transpose_gu_last()
                onesL = jnp.ones((16, 128), BF)
                for n in range(2 * NFB + 1):
                    a = None
                    for mb in range(NMB):
                        a = _acc(a, _dot(onesL, _tile(guT_u, (n * NMB + mb) * 64))[0:8])
                    cs_scr[pl.ds(n * 8, 8), :] = a
                wait(g_o1)
                start(g_d23a)
            def flhs(h):
                hh, r = divmod(h, 16)
                return jnp.broadcast_to(ctx[hh][r:r + 1, :], (16, 128)).astype(BF)
            FV = opts.get('fv', ())
            acc = [None] * NMB
            vlo = [None] * NMB
            vhi = [None] * NMB

            mts = {}

            def f_group(h, k, dep):
                if h not in mts:
                    L = flhs(h)
                    mts[h] = pltpu.bitcast(jnp.concatenate([L] * 8, axis=0).T, U32)
                mk = mts[h][8 * k:8 * k + 8]
                if dep is not None:
                    mk = jnp.where(always, mk, pltpu.bitcast(dep, U32))
                mlo, mhi = unpack(mk)
                for mb in range(NMB):
                    wlo, whi = unpack(wo_u[pl.ds(mb * (SK // 2) + h * 64 + 8 * k, 8), :])
                    vlo[mb] = _acc(vlo[mb], wlo * mlo + whi * mhi)

            DEPD = opts.get('depd', 2)
            RHO = opts.get('rho', 1.0)

            def run_mixed(mh, vh):
                Lc = {}

                def f_tile(h, mb):
                    def fn():
                        if h not in Lc:
                            Lc[h] = flhs(h)
                        acc[mb] = _acc(acc[mb], _dot(Lc[h], _tile(wo_u, mb * (SK // 2) + h * 64))[0:8])
                        return acc[mb]
                    return fn

                def f_grp(h, k):
                    def fn(dep):
                        f_group(h, k, dep)
                        return vlo[NMB - 1]
                    return fn
                paced([f_tile(h, mb) for h in mh for mb in range(NMB)], [f_grp(h, k) for h in vh for k in range(8)], DEPD, RHO)
            run_mixed([h for h in range(NH1) if h not in FV], [h for h in range(NH1) if h in FV])
            if first:
                wait(g_o2)
                start(g_d23b)
            assert all(h < NH1 for h in FV)
            Ls = {h: flhs(h) for h in range(NH1, 32) if h not in FV}
            x1 = []
            for mb in range(NMB):
                for h in Ls:
                    acc[mb] = _acc(acc[mb], _dot(Ls[h], _tile(wo_u, mb * (SK // 2) + h * 64))[0:8])
                a = acc[mb]
                if FV:
                    a = a + jnp.sum(vlo[mb], axis=0, keepdims=True)
                x1.append(x[mb] + a)
            GV = tuple(opts.get('gv', ()))
            L = [_rep16(x1[b]) for b in range(NMB)]
            mean, inv = _stats(x1)
            xn1 = [(x1[b] - mean) * inv for b in range(NMB)]
            rr = xn1[0] * wr_rows[0]
            for b in range(1, NMB):
                rr = rr + xn1[b] * wr_rows[b]
            r = jnp.sum(rr, axis=1, keepdims=True)
            sig = 1.0 / (1.0 + jnp.exp(-r))

            def fin(a, n):
                return (a - mean * cs_scr[pl.ds(n * 8, 8), :]) * inv
            hs = [None] * (NFB + 1)
            sigt = [sig]
            accs = {}
            mfb = [fb for fb in range(NFB) if fb not in GV]
            mxu_fns = []

            HV = tuple(opts.get('hv', ()))
            mth = {}

            def g_tile(fb, which, mb):
                def fn():
                    o = _dot(L[mb], _tile(guT_u, gu_index(which, fb, mb) * 64))[0:8]
                    accs[fb, which] = _acc(accs.get((fb, which)), o)
                    res = o if opts.get('rawdep', 0) else accs[fb, which]
                    if which == 1 and mb == NMB - 1 and opts.get('early_hs', 1):
                        hs[fb] = silu(fin(accs[fb, 0], fb)) * fin(accs[fb, 1], NFB + fb)
                        if opts.get('sigtie', 0) and fb == mfb[opts.get('sigtie', 0)]:
                            hs[fb] = jnp.where(always, hs[fb], jnp.broadcast_to(sig, (8, 128)))
                        if fb in HV and not first:
                            mth[fb] = pltpu.bitcast(jnp.concatenate([_rep16(hs[fb])] * 8, axis=0).T, U32)
                    return res
                return fn
            for mb in range(NMB):
                for fb in mfb[:G1]:
                    for which in range(2):
                        mxu_fns.append(g_tile(fb, which, mb))
            for fb in mfb[G1:]:
                for which in range(2):
                    for mb in range(NMB):
                        mxu_fns.append(g_tile(fb, which, mb))
            vacc = {}
            mtg = {}

            def g_group(mb, k, which):
                def fn(dep):
                    if mb not in mtg:
                        mtg[mb] = pltpu.bitcast(jnp.concatenate([_rep16(x1[mb])] * 8, axis=0).T, U32)
                    mlo, mhi = unpack(tie(mtg[mb][8 * k:8 * k + 8], dep))
                    for fb in GV:
                        wlo, whi = unpack(guT_u[pl.ds(gu_index(which, fb, mb) * 64 + 8 * k, 8), :])
                        vacc[fb, which] = _acc(vacc.get((fb, which)), wlo * mlo + whi * mhi)
                    return vacc[GV[-1], which]
                return fn
            vpu_fns = [g_group(mb, k, which) for mb in range(NMB) for k in range(8) for which in range(2)] if GV else []
            lastacc = [None]

            def gl_tile(mb):
                def fn():
                    lastacc[0] = _acc(lastacc[0], _dot(L[mb], _tile(guT_u, (2 * NFB * NMB + mb) * 64))[0:8])
                    res = lastacc[0]
                    if mb == NMB - 1:
                        a = fin(res, 2 * NFB)
                        sw = pltpu.roll(a, 64, axis=1)
                        g = jnp.where(lane < 64, a, sw)
                        u = jnp.where(lane < 64, sw, a)
                        hs[NFB] = silu(g) * u
                    return res
                return fn
            mxu_fns += [gl_tile(mb) for mb in range(NMB)]

            def finish_mxu_blocks():
                for fb in mfb:
                    if hs[fb] is None:
                        hs[fb] = silu(fin(accs[fb, 0], fb)) * fin(accs[fb, 1], NFB + fb)

            def finish_vpu_blocks():
                for i, fb in enumerate(GV):
                    gu = []
                    for which in range(2):
                        raw = jnp.sum(vacc[fb, which], axis=0, keepdims=True)
                        gu.append(fin(raw, which * NFB + fb))
                    hs[fb] = silu(gu[0]) * gu[1]
            if not fuse_h:
                paced(mxu_fns, vpu_fns, opts.get('gdepd', 2), opts.get('grho', 1.0))
                finish_mxu_blocks()
                finish_vpu_blocks()
                return x1, xn1, sig, hs, mean
            h_mxu, h_vpu, h_done = h_streams(hs, mth, finish_mxu_blocks)
            ng = len(vpu_fns)

            def last_g_group(fn):
                def w(dep):
                    r = fn(dep)
                    finish_vpu_blocks()
                    return r
                return w
            if vpu_fns:
                vpu_fns[-1] = last_g_group(vpu_fns[-1])
            paced(mxu_fns + h_mxu, vpu_fns + h_vpu, opts.get('gdepd', 2), opts.get('grho', 1.0))
            return x1, xn1, sig, h_done(), None

        def h_last_lhs(hl):
            z = jnp.zeros_like(hl)
            ev = jnp.where(lane < 64, hl, z)
            od = jnp.where(lane < 64, z, hl)
            return _rep16(jnp.where(sub % 2 == 0, ev, od))

        def h_last_tile(L, mb, mb2):
            r0 = NFB * 64
            t = jnp.concatenate([wd_u[pl.ds(mb * (F // 2) + r0, 32), :], wd_u[pl.ds(mb2 * (F // 2) + r0, 32), :]], axis=0)
            return _dot(L, pltpu.bitcast(t, BF))[0:8]

        def h_streams(hs, mth, finish_mxu_blocks):
            GV = tuple(opts.get('gv', ()))
            HV = tuple(opts.get('hv', ()))
            acc = [None] * NMB
            order = [fb for fb in range(NFB) if fb not in GV] + [NFB] + list(GV)
            mxu_fns = []
            Lc = {}

            def h_tile(fb, mb):
                def fn():
                    if fb not in Lc:
                        finish_mxu_blocks()
                        Lc[fb] = _rep16(hs[fb])
                    o = _dot(Lc[fb], _tile(wd_u, mb * (F // 2) + fb * 64))[0:8]
                    acc[mb] = _acc(acc[mb], o)
                    return o if opts.get('rawdep', 0) else acc[mb]
                return fn

            def h_last(mb):
                def fn():
                    if NFB not in Lc:
                        Lc[NFB] = h_last_lhs(hs[NFB])
                    mb2 = min(mb + 1, NMB - 1)
                    o = h_last_tile(Lc[NFB], mb, mb2)
                    acc[mb] = acc[mb] + jnp.broadcast_to(o[0:1], (8, 128))
                    if mb2 != mb:
                        acc[mb2] = acc[mb2] + jnp.broadcast_to(o[1:2], (8, 128))
                    return acc[mb]
                return fn
            for fb in order:
                if fb in HV:
                    continue
                if fb == NFB:
                    mxu_fns += [h_last(mb) for mb in range(0, NMB, 2)]
                else:
                    mxu_fns += [h_tile(fb, mb) for mb in range(NMB)]
            vacc = [None] * NMB

            def h_group(fb, k):
                def fn(dep):
                    if fb not in mth:
                        finish_mxu_blocks()
                        mth[fb] = pltpu.bitcast(jnp.concatenate([_rep16(hs[fb])] * 8, axis=0).T, U32)
                    mlo, mhi = unpack(tie(mth[fb][8 * k:8 * k + 8], dep))
                    for mb in range(NMB):
                        wlo, whi = unpack(wd_u[pl.ds(mb * (F // 2) + fb * 64 + 8 * k, 8), :])
                        vacc[mb] = _acc(vacc[mb], wlo * mlo + whi * mhi)
                    return vacc[NMB - 1]
                return fn

            def done():
                if HV:
                    return [acc[mb] + jnp.sum(vacc[mb], axis=0, keepdims=True) for mb in range(NMB)]
                return acc
            return mxu_fns, [h_group(fb, k) for fb in HV for k in range(8)], done

        def next_layer_head(x1, xn1, sig, hs, first, mean1):
            Lh = [_rep16(hs[fb]) for fb in range(NFB)]
            Ll = h_last_lhs(hs[NFB])
            acc = [None] * NMB
            x2 = [None] * NMB
            q = [None, None]

            def hpart(fbs, mbs):
                for fb in fbs:
                    for mb in mbs:
                        acc[mb] = _acc(acc[mb], _dot(Lh[fb], _tile(wd_u, mb * (F // 2) + fb * 64))[0:8])

            def hlast(mb, mb2):
                o = h_last_tile(Ll, mb, mb2)
                acc[mb] = acc[mb] + jnp.broadcast_to(o[0:1], (8, 128))
                if mb2 != mb:
                    acc[mb2] = acc[mb2] + jnp.broadcast_to(o[1:2], (8, 128))

            NDEF = opts.get('ndef', 8)
            ds = {}

            def finish_x(mb):
                x2[mb] = x1[mb] + xn1[mb] + acc[mb] * sig
                ds[mb] = dup_bits(x2[mb])

            def ablock(mb, rs, hhs=(0, 1)):
                for r in rs:
                    l0 = xlhs(ds[mb], r, XQ)
                    for hh in hhs:
                        q[hh] = _acc(q[hh], _dot(l0, xtile(wq_u, 16 * mb + r, hh)))

            if first:
                wait(g_d01)
                start(g_d4a)
            hpart(range(NFB), (0, 1))
            hlast(0, 1)
            finish_x(0)
            finish_x(1)
            ablock(0, range(16))
            ablock(1, range(16))
            if first:
                wait(g_d23a)
            hpart(range(FS23), (2, 3))
            if first:
                wait(g_d23b)
            hpart(range(FS23, NFB), (2,))
            hlast(2, 2)
            hpart(range(FS23, NFB), (3,))
            hlast(3, 3)
            finish_x(2)
            finish_x(3)
            if opts.get('av', 0) and opts.get('mtearly', 1):
                mt_scr[...] = jnp.concatenate([_rep16(x2[3])] * 8, axis=0).T
            ablock(2, range(16))
            ablock(3, range(16 - NDEF))
            H1PRE = opts.get('h1pre', 0)
            ablock(3, range(16 - NDEF, 16 - NDEF + H1PRE), hhs=(1,))
            mb = NMB - 1
            if first:
                wait(g_d4a)
            hpart(range(FS4), (mb,))
            if first and g_d4b:
                wait(g_d4b)
            if first and opts.get('stop', 0):
                return x2[:4] + [acc[mb]], q
            lcache = {}
            AV = opts.get('av', 0)
            seg1 = [lambda fb=fb: hpart([fb], (mb,)) or acc[mb] for fb in range(FS4, NFB)]
            seg1.append(lambda: hlast(mb, mb) or acc[mb])

            def a_tile(blk, r, hh):
                def fn():
                    if not opts.get('lcache', 0) or (blk, r) not in lcache:
                        lcache[blk, r] = xlhs(ds[blk], r, XQ)
                        if blk == NMB - 1 and hh == 0 and r == opts.get('sttie', -1):
                            inv_b = jnp.broadcast_to(st[0][1], (8, 128))
                            lcache[blk, r] = pltpu.bitcast(tie(pltpu.bitcast(lcache[blk, r], U32), inv_b), BF)
                    o = _dot(lcache[blk, r], xtile(wq_u, 16 * blk + r, hh))
                    q[hh] = _acc(q[hh], o)
                    return o[0:8]
                return fn
            seg1 += [a_tile(3, r, 0) for r in range(16 - NDEF, 16)]

            st = []

            def fx():
                finish_x(mb)
                if opts.get('stshift', 1):
                    st.append(_stats_shift(x2, mean1))
                else:
                    st.append(_stats(x2))
                return a_tile(mb, 0, 0)()
            seg1.append(fx)
            seg1 += [a_tile(mb, r, 0) for r in range(1, 16)]
            vq = {}
            mt3 = []

            def av_group(g2):
                def fn(dep):
                    if not mt3 and not opts.get('mtearly', 1):
                        mt3.append(1)
                        mt_scr[...] = jnp.concatenate([_rep16(x2[3])] * 8, axis=0).T
                    for i in (2 * g2, 2 * g2 + 1):
                        row = mt_u[pl.ds(i, 1), :]
                        mp = tie(jnp.broadcast_to(row, (8, 128)), dep if i % 2 == 0 else None)
                        m0, m1 = unpack(mp)
                        w0l, w0h = unpack(wq_u[pl.ds((3 * 128 + 2 * i) * 16 + 8, 8), :])
                        w1l, w1h = unpack(wq_u[pl.ds((3 * 128 + 2 * i + 1) * 16 + 8, 8), :])
                        vq['e'] = _acc(vq.get('e'), w0l * m0 + w1l * m1)
                        vq['o'] = _acc(vq.get('o'), w0h * m0 + w1h * m1)
                    return vq['e']
                return fn
            r_v = list(range(16 - AV, 16))
            vfns = [av_group(2 * r + j) for r in r_v for j in range(2)]
            nsplit = opts.get('avsplit', len(vfns))
            paced(seg1, vfns[:nsplit], opts.get('adepd', 2), opts.get('arho', 1.0), opts.get('askip', 0))
            tail = [a_tile(3, r, 1) for r in range(16 - NDEF + H1PRE, 16) if r not in r_v]
            for r in range(16 - NDEF):
                assert r not in r_v
            tail += [a_tile(mb, r, 1) for r in range(16)]
            vtail = vfns[nsplit:]
            if opts.get('stop', 0):
                for fn in tail:
                    fn()
            return x2, q, tail, vtail, vq, st[0]

        wait(g_q)
        start(g_uv)
        xrow = xb[0].astype(F32)
        x = [jnp.broadcast_to(xrow[:, b * 128:(b + 1) * 128], (8, 128)) for b in range(NMB)]
        wrf = wrb[...].astype(F32)
        wr_rows = [jnp.broadcast_to(wrf[b:b + 1, :], (8, 128)) for b in range(NMB)]
        always = (pltpu.bitcast(wr_rows[0], U32) | np.uint32(1)) != np.uint32(0)
        csq = colsum_q()
        q = [None, None]
        for mb in range(NMB):
            d = dup_bits(x[mb])
            xblock([d, d], wq_u, mb, q, mask=XQ)

        def make_finish(x, vq=None, st=None):
            mean, inv = _stats(x) if st is None else st
            def fin_q(raw, cs, hh):
                if vq and hh == 1:
                    raw = raw + jnp.concatenate([vq['e'], vq['o']], axis=0)
                return (raw - mean[0:1] * cs) * inv[0:1]
            return fin_q
        wait(g_uk)
        start(g_g)
        relayout_uk()
        ctx = attention(q, make_finish(x), csq, True)
        x1, xn1, sig, hs, mean1 = mix(x, ctx, True)
        for it in range(1 + extra):
            x, q, tail, vtail, vq, st2 = next_layer_head(x1, xn1, sig, hs, it == 0, mean1)
            if opts.get('stop', 0):
                out = jnp.concatenate([xb_[0:1] + q[0][0:1] + q[1][0:1] for xb_ in x], axis=1)
                o_ref[...] = out.astype(BF).reshape(1, 1, M)
                return
            ctx = attention(q, make_finish(x, vq, st2), csq, False, tail, vtail)
            if it < extra:
                x1, xn1, sig, hs, mean1 = mix(x, ctx, False)
            else:
                x1, xn1, sig, acc, _ = mix(x, ctx, False, fuse_h=True)
        xo = [x1[b] + xn1[b] + acc[b] * sig for b in range(NMB)]
        out = jnp.concatenate([xb_[0:1] for xb_ in xo], axis=1)
        o_ref[...] = out.astype(BF).reshape(1, 1, M)

    scratch = [
        pltpu.VMEM((1, 1, M), BF),
        pltpu.VMEM((NMB, 128), BF),
        pltpu.VMEM((M * H, D), BF),
        pltpu.VMEM((DC * H, D), BF),
        pltpu.VMEM((DC * H, D), BF),
        pltpu.VMEM((NCB * SK, 128), BF),
        pltpu.VMEM((NCB * SK, 128), BF),
        pltpu.VMEM((DC * H, D), BF),
        pltpu.VMEM((NMB * SK, 128), BF),
        pltpu.VMEM((F, M), BF),
        pltpu.VMEM((F, M), BF),
        pltpu.VMEM(((2 * NFB * NMB + NMB) * 128, 128), BF),
        pltpu.VMEM((NMB * F, 128), BF),
        pltpu.VMEM((H, SK), F32),
        pltpu.VMEM(((2 * NFB + 1) * 8, 128), F32),
        pltpu.VMEM((128, 128), BF),
        pltpu.SemaphoreType.DMA((3,)),
    ]

    def fn(A_x, A_c_kv, A_w_q, A_w_uk, A_w_uv, A_w_o, B_x, B_w_r, B_w_gate, B_w_up, B_w_down):
        return pl.pallas_call(
            kernel,
            out_shape=jax.ShapeDtypeStruct((1, 1, M), BF),
            in_specs=[pl.BlockSpec(memory_space=pltpu.HBM)] * 10,
            out_specs=pl.BlockSpec(memory_space=pltpu.VMEM),
            scratch_shapes=scratch,
            compiler_params=pltpu.CompilerParams(vmem_limit_bytes=100 * 1024 * 1024, flags=opts.get('flags', None)),
        )(A_x, B_w_r.reshape(NMB, 128), A_w_q.reshape(M * H, D), A_w_uk.reshape(DC * H, D),
          A_c_kv.reshape(SK, DC), A_w_uv.reshape(DC * H, D), A_w_o.reshape(H * D, M),
          B_w_gate.T, B_w_up.T, B_w_down)
    return fn


@jax.jit
def pallas_interleave_layers__compressed_kv_cla__moe_arch_mod__decode_kernel(
    A_x: jax.Array,
    A_c_kv: jax.Array,
    A_w_q: jax.Array,
    A_w_uk: jax.Array,
    A_w_uv: jax.Array,
    A_w_o: jax.Array,
    B_x: jax.Array,
    B_w_r: jax.Array,
    B_w_gate: jax.Array,
    B_w_up: jax.Array,
    B_w_down: jax.Array,
):
    fn = build({'ndef':16,'fs4':0,'nh1':28,'fv':(1,3,5,7,9,11,13,15,17,19),'gv':(9,10,11,12),'hv':(0,1,2),'depd':1,'grho':1.2,'g1':3,'sigtie':5,'nb2':8,'bv':(5,6,7),'bahead':0,'bskip':20,'av':0,'h1pre':16,'sttie':8,'bdepd':4})
    return fn(A_x, A_c_kv, A_w_q, A_w_uk, A_w_uv, A_w_o, B_x, B_w_r, B_w_gate, B_w_up, B_w_down)
```

```python
import functools
import contextlib
import numpy as np
import jax
import jax.numpy as jnp
from jax import lax
import jax.experimental.pallas as pl
import jax.experimental.pallas.tpu as pltpu

M, H, D, DC, SK, F = 640, 32, 128, 512, 4096, 1728
NMB = M // 128
NCB = DC // 128
NKB = SK // 128
NFB = F // 128
FREM = F - NFB * 128
LOG2E = 1.4426950408889634
EPS = 1e-5
BF = jnp.bfloat16
F32 = jnp.float32
U32 = jnp.uint32


def _dot(a, b):
    return jnp.dot(a, b, preferred_element_type=F32)


def _tile(ref_u32, r0):
    return pltpu.bitcast(ref_u32[pl.ds(r0, 64), :], BF)


def _iota(shape, ax):
    return lax.broadcasted_iota(jnp.int32, shape, ax)


def _pack_rows(v):
    return pltpu.bitcast(v.astype(BF), U32)


def _stats(x):
    s = x[0]
    for b in range(1, NMB):
        s = s + x[b]
    mean = jnp.sum(s, axis=1, keepdims=True) * (1.0 / M)
    xc = [xb - mean for xb in x]
    v = xc[0] * xc[0]
    for b in range(1, NMB):
        v = v + xc[b] * xc[b]
    var = jnp.sum(v, axis=1, keepdims=True) * (1.0 / M)
    return mean, lax.rsqrt(var + EPS)


def _stats_shift(x, shift):
    d = [xb - shift for xb in x]
    s1 = d[0]
    s2 = d[0] * d[0]
    for b in range(1, NMB):
        s1 = s1 + d[b]
        s2 = s2 + d[b] * d[b]
    m1 = jnp.sum(s1, axis=1, keepdims=True) * (1.0 / M)
    m2 = jnp.sum(s2, axis=1, keepdims=True) * (1.0 / M)
    var = jnp.maximum(m2 - m1 * m1, 0.0)
    return shift + m1, lax.rsqrt(var + EPS)


def _rep16(v):
    return jnp.concatenate([v, v], axis=0).astype(BF)


def unpack(w):
    lo = pltpu.bitcast(w << 16, F32)
    hi = pltpu.bitcast(w & np.uint32(0xFFFF0000), F32)
    return lo, hi


def _acc(a, o):
    return o if a is None else a + o


def build(opts=None):
    opts = dict(opts or {})
    WO_RC = opts.get('wo_rc', 8)
    WD_RC = opts.get('wd_rc', 12)
    WD_SPLIT = opts.get('wd_split', 9)
    NA = opts.get('na', 8)
    NB2 = opts.get('nb2', 8)
    G1 = opts.get('g1', 3)
    scoped = opts.get('scoped', False)
    extra = opts.get('extra', 0)

    def scope(name):
        if scoped:
            return jax.named_scope(name)
        import contextlib
        return contextlib.nullcontext()

    def kernel(x_hbm, wr_hbm, wq_hbm, wuk_hbm, ckv_hbm, wuv_hbm, wo_hbm, wg_hbm, wu_hbm, wd_hbm,
               o_ref,
               xb, wrb, wq, wuk, ukT, ckv, ckvT, wuv, wo, wg, wu, guT, wd, s_scr, cs_scr, mt_scr, sems):
        def cp(src, dst, s):
            return pltpu.make_async_copy(src, dst, sems.at[s])
        g_q = [cp(wq_hbm, wq, 0), cp(x_hbm, xb, 0), cp(wr_hbm, wrb, 0)]
        g_uk = [cp(wuk_hbm, wuk, 1)]
        g_ckv = [cp(ckv_hbm.at[:, pl.ds(j * 128, 128)], ckv.at[pl.ds(j * SK, SK)], 2) for j in range(NCB)]
        g_uv = [cp(wuv_hbm, wuv, 0)]
        g_g = [cp(wg_hbm, wg, 1)]
        g_u = [cp(wu_hbm, wu, 2)]
        NH1 = opts.get('nh1', 24)
        g_o1, g_o2 = [], []
        for r in range(WO_RC):
            n = SK // WO_RC
            for j in range(NMB):
                p1 = r * n < NH1 * D
                (g_o1 if p1 else g_o2).append(
                    cp(wo_hbm.at[pl.ds(r * n, n), pl.ds(j * 128, 128)], wo.at[pl.ds(j * SK + r * n, n)], 0 if p1 else 1))
        nu = F // 64
        bounds = [(nu * j // WD_RC) * 64 for j in range(WD_RC + 1)]

        def slab(a, b, j, s):
            return cp(wd_hbm.at[pl.ds(a, b - a), pl.ds(j * 128, 128)], wd.at[pl.ds(j * F + a, b - a)], s)
        RS = opts.get('rs34', 9)
        FS34 = bounds[RS] // 128
        g_d012 = [slab(bounds[r], bounds[r + 1], j, 2) for r in range(WD_RC) for j in (0, 1, 2)]
        g_d34a = [slab(bounds[r], bounds[r + 1], j, 0) for r in range(RS) for j in (3, 4)]
        g_d34b = [slab(bounds[r], bounds[r + 1], j, 1) for r in range(RS, WD_RC) for j in (3, 4)]

        def start(grp):
            for c in grp:
                c.start()

        wcount = [0]

        def wait(grp):
            with scope('wait%02d' % wcount[0]):
                for c in grp:
                    c.wait()
            wcount[0] += 1

        start(g_q)
        start(g_uk)
        start(g_ckv)

        if opts.get('dmaonly', 0):
            wait(g_q); start(g_uv); wait(g_uk); start(g_g); wait(g_ckv); start(g_u); wait(g_uv); start(g_o1)
            wait(g_g); start(g_o2); wait(g_u); start(g_d012); wait(g_o1); start(g_d34a); wait(g_o2); start(g_d34b); wait(g_d012); wait(g_d34a); wait(g_d34b)
            o_ref[...] = xb[...]
            return
        lane = _iota((8, 128), 1)
        sub = _iota((8, 128), 0)
        h16 = lane % 16
        XM = jnp.where(h16 == 2 * sub, np.uint32(0x0000FFFF),
                       jnp.where(h16 == 2 * sub + 1, np.uint32(0xFFFF0000), np.uint32(0)))
        rlo, rhi = 2 * sub, 2 * sub + 1
        hlo = jnp.where(rlo < 8, 2 * rlo, 2 * (rlo - 8) + 1)
        hhi = jnp.where(rhi < 8, 2 * rhi, 2 * (rhi - 8) + 1)
        XQ = (jnp.where(h16 == hlo, np.uint32(0x0000FFFF), np.uint32(0))
              | jnp.where(h16 == hhi, np.uint32(0xFFFF0000), np.uint32(0)))
        idx16 = lane // 16
        PM = jnp.where(lane % 2 == 0, np.uint32(0x0000FFFF), np.uint32(0xFFFF0000))
        idx2 = lane // 2

        wq_u = wq.bitcast(U32)
        wuk_u = wuk.bitcast(U32)
        wuv_u = wuv.bitcast(U32)
        mt_u = mt_scr.bitcast(U32)
        ukT_u = ukT.bitcast(U32)
        ckv_u = ckv.bitcast(U32)
        ckvT_u = ckvT.bitcast(U32)
        wo_u = wo.bitcast(U32)
        guT_u = guT.bitcast(U32)
        wd_u = wd.bitcast(U32)

        def xtile(w_u, g, hh):
            rows = [w_u[pl.ds((8 * g + j) * 16 + 8 * hh, 8), :] for j in range(8)]
            return pltpu.bitcast(jnp.concatenate(rows, axis=0), BF)

        def xlhs(src, r, mask=None):
            mask = XM if mask is None else mask
            return pltpu.bitcast(jnp.take_along_axis(src, idx16 + 8 * r, axis=1) & mask, BF)

        def xblock(srcs, w_u, blk, acc, hhs=(0, 1), mask=None):
            for r in range(16):
                l0 = None
                for hh in hhs:
                    if l0 is None or srcs[hh] is not srcs[hhs[0]]:
                        l0 = xlhs(srcs[hh], r, mask)
                    acc[hh] = _acc(acc[hh], _dot(l0, xtile(w_u, 16 * blk + r, hh)))

        def dup_bits(v):
            u = pltpu.bitcast(v.astype(BF).astype(F32), U32)
            return u | (u >> 16)

        def colsum_q():
            if opts.get('no_cs', 0): return [jnp.zeros((16,128),F32)]*2
            l0 = pltpu.bitcast(XQ & np.uint32(0x3F803F80), BF)
            acc = [None, None]
            for g in range(M // 8):
                for hh in range(2):
                    acc[hh] = _acc(acc[hh], _dot(l0, xtile(wq_u, g, hh)))
            return acc

        def relayout_uk():
            if opts.get('no_uk', 0): return
            for hp in range(16):
                for cb in range(NCB):
                    s = wuk_u[pl.ds(128 * cb * 16 + hp, 128, stride=16), :]
                    ukT[pl.ds((hp * NCB + cb) * 256, 256), :] = pltpu.bitcast(s.T, BF)

        def transpose_ckv():
            if opts.get('no_ckv', 0): return
            for cb in range(NCB):
                for kb in range(NKB):
                    t = ckv[pl.ds(cb * SK + kb * 128, 128), :]
                    ckvT[pl.ds((cb * NKB + kb) * 128, 128), :] = t.T

        def gu_index(which, fb, mb):
            return (which * NFB + fb) * NMB + mb

        def transpose_gu(which, src):
            if opts.get('no_gu', 0): return
            for fb in range(NFB):
                for mb in range(NMB):
                    t = src[pl.ds(fb * 128, 128), pl.ds(mb * 128, 128)]
                    guT[pl.ds(gu_index(which, fb, mb) * 128, 128), :] = t.T

        def transpose_gu_last():
            for mb in range(NMB):
                t = jnp.concatenate([wg[pl.ds(NFB * 128, FREM), pl.ds(mb * 128, 128)],
                                     wu[pl.ds(NFB * 128, FREM), pl.ds(mb * 128, 128)]], axis=0)
                guT[pl.ds((2 * NFB * NMB + mb) * 128, 128), :] = t.T

        def b_block(L, hh, cb):
            acc = None
            for hp8 in range(8):
                hp = hh * 8 + hp8
                for kh in range(2):
                    Lm = pltpu.bitcast(jnp.where(sub == hp8, L[kh], np.uint32(0)), BF)
                    acc = _acc(acc, _dot(Lm, _tile(ukT_u, (hp * NCB + cb) * 128 + 64 * kh)))
            return acc

        def b_lhs(qh):
            qp = _pack_rows(qh)
            return [jnp.take_along_axis(qp, idx2 + 64 * kh, axis=1) & PM for kh in range(2)]

        CEXP = (D ** -0.5) * LOG2E

        def sblk(kb):
            return s_scr.at[:, kb * 128:(kb + 1) * 128]

        def attention(q_raw, finish_q, csq, first, pre_fns=(), pre_v=()):
            BV = tuple(opts.get('bv', ()))
            qa = [[None] * NCB for _ in range(2)]
            qps = {}

            def get_qp(hh):
                if hh not in qps:
                    qf = finish_q(q_raw[hh], csq[hh], hh)
                    qps[hh] = pltpu.bitcast(pltpu.pack_elementwise([qf[0:8], qf[8:16]], packed_dtype=BF), U32)
                return qps[hh]
            Lb = {}

            def b_tile(hh, cb, hp8, kh):
                def fn():
                    if hh not in Lb:
                        qp = get_qp(hh)
                        Lb[hh] = [jnp.take_along_axis(qp, idx2 + 64 * k2, axis=1) & PM for k2 in range(2)]
                    Lm = pltpu.bitcast(jnp.where(sub == hp8, Lb[hh][kh], np.uint32(0)), BF)
                    o = _dot(Lm, _tile(ukT_u, ((hh * 8 + hp8) * NCB + cb) * 128 + 64 * kh))
                    qa[hh][cb] = _acc(qa[hh][cb], o)
                    return o[0:8]
                return fn

            def b_fns(hh, cb):
                return [b_tile(hh, cb, hp8, kh) for hp8 in range(8) if (hh * 8 + hp8) not in BV for kh in range(2)]
            mtb = {}
            blo, bhi = {}, {}

            def mk_mtb(hp):
                if hp not in mtb:
                    qp = get_qp(hp // 8)
                    mtb[hp] = jnp.broadcast_to(qp[hp % 8:hp % 8 + 1, :], (128, 128)).T

            def b_group(hp, k):
                def fn(dep):
                    mk_mtb(hp)
                    i = BV.index(hp)
                    for ahead in range(1, opts.get('bahead', 0) + 1):
                        if i + ahead < len(BV):
                            mk_mtb(BV[i + ahead])
                    mlo, mhi = unpack(tie(mtb[hp][8 * k:8 * k + 8], dep))
                    for cb in range(NCB):
                        wlo, whi = unpack(ukT_u[pl.ds((hp * NCB + cb) * 128 + 8 * k, 8), :])
                        blo[hp, cb] = _acc(blo.get((hp, cb)), wlo * mlo)
                        bhi[hp, cb] = _acc(bhi.get((hp, cb)), whi * mhi)
                    return blo[hp, NCB - 1]
                return fn
            if BV:
                mk_mtb(BV[0])
                if len(BV) > 1 and opts.get('bahead', 0):
                    mk_mtb(BV[1])
            mfns = list(pre_fns)
            for cb in range(NCB):
                mfns += b_fns(0, cb)
            for cb in range(NCB - 1):
                mfns += b_fns(1, cb)
            paced(mfns, list(pre_v) + [b_group(hp, k) for hp in BV for k in range(16)], opts.get('bdepd', 2), opts.get('brho', 1.0), opts.get('bskip', 0))
            for hp in BV:
                hh, hp8 = divmod(hp, 8)
                v, r0 = hp8 // 4, 2 * (hp8 % 4)
                for cb in range(NCB):
                    lo, hi = blo[hp, cb], bhi[hp, cb]
                    u = jnp.where(sub % 2 == 0, lo + pltpu.roll(lo, 7, axis=0), hi + pltpu.roll(hi, 1, axis=0))
                    u = u + pltpu.roll(u, 2, axis=0)
                    u = u + pltpu.roll(u, 4, axis=0)
                    parts = [qa[hh][cb][0:8], qa[hh][cb][8:16]]
                    parts[v] = jnp.where((sub == r0) | (sub == r0 + 1), u, parts[v])
                    qa[hh][cb] = jnp.concatenate(parts, axis=0)

            def c_lhs(cb):
                return jnp.concatenate([qa[0][cb], qa[1][cb]], axis=0).astype(BF)
            if first:
                wait(g_ckv)
                start(g_u)
                transpose_ckv()
            lhs = [None] * NCB
            lhs[0] = c_lhs(0)
            for kb in range(NA):
                sblk(kb)[...] = _dot(lhs[0], _tile(ckvT_u, (0 * NKB + kb) * 64))
            for fn in b_fns(1, NCB - 1):
                fn()
            mx = None
            for cb in range(1, NCB):
                lhs[cb] = c_lhs(cb)
                for kb in range(NA):
                    s = sblk(kb)[...] + _dot(lhs[cb], _tile(ckvT_u, (cb * NKB + kb) * 64))
                    sblk(kb)[...] = s
                    if cb == NCB - 1:
                        mx = s if mx is None else jnp.maximum(mx, s)
            mA = jnp.max(mx, axis=1, keepdims=True)
            for kb in range(NA, NKB):
                s = None
                for cb in range(NCB):
                    s = _acc(s, _dot(lhs[cb], _tile(ckvT_u, (cb * NKB + kb) * 64)))
                sblk(kb)[...] = s
                mx = jnp.maximum(mx, s)
            mB = jnp.max(mx, axis=1, keepdims=True)
            acc = [None] * NCB
            l = None
            for kb in range(NA):
                p = jnp.exp2((sblk(kb)[...] - mA) * CEXP)
                l = _acc(l, p)
                pb = p.astype(BF)
                for cb in range(NCB):
                    acc[cb] = _acc(acc[cb], _dot(pb, _tile(ckv_u, cb * (SK // 2) + kb * 64)))
            alpha = jnp.exp2((mA - mB) * CEXP)
            acc = [a * alpha for a in acc]
            l = l * alpha
            for kb in range(NA, NKB - NB2):
                p = jnp.exp2((sblk(kb)[...] - mB) * CEXP)
                l = l + p
                pb = p.astype(BF)
                for cb in range(NCB):
                    acc[cb] = acc[cb] + _dot(pb, _tile(ckv_u, cb * (SK // 2) + kb * 64))
            pbs = []
            for kb in range(NKB - NB2, NKB):
                p = jnp.exp2((sblk(kb)[...] - mB) * CEXP)
                l = l + p
                pbs.append(p.astype(BF))
            linv = 1.0 / jnp.sum(l, axis=1, keepdims=True)
            srcs = []
            for cb in range(NCB):
                for i, kb in enumerate(range(NKB - NB2, NKB)):
                    acc[cb] = acc[cb] + _dot(pbs[i], _tile(ckv_u, cb * (SK // 2) + kb * 64))
                cc = acc[cb] * linv
                srcs.append([_pack_rows(cc[0:16]), _pack_rows(cc[16:32])])
            if first:
                wait(g_uv)
                start(g_o1)
            ctx = [None, None]
            for cb in range(NCB - 1):
                xblock(srcs[cb], wuv_u, cb, ctx)
            xblock(srcs[NCB - 1], wuv_u, NCB - 1, ctx, hhs=(0,))
            xblock(srcs[NCB - 1], wuv_u, NCB - 1, ctx, hhs=(1,))
            return ctx

        def paced(mxu_fns, vpu_fns, depd, rho_scale=1.0, skip=0):
            rho = len(vpu_fns) / max(1, len(mxu_fns) - skip) * rho_scale
            SELF = opts.get('self', 0)
            res = []
            vres = []
            j = 0

            def run_v(t):
                if SELF:
                    dep = vres[j - SELF] if j >= SELF else None
                else:
                    dep = res[max(t - depd, 0)] if depd >= 0 else None
                vres.append(vpu_fns[j](dep))
            for t, fn in enumerate(mxu_fns):
                res.append(fn())
                while j < len(vpu_fns) and j < rho * (t + 1 - skip):
                    run_v(t)
                    j += 1
            while j < len(vpu_fns):
                run_v(len(mxu_fns) - 1)
                j += 1

        def tie(v, dep):
            if dep is None:
                return v
            return jnp.where(always, v, pltpu.bitcast(dep, U32))

        def silu(g):
            return g / (1.0 + jnp.exp(-g))

        ones8 = jnp.ones((8, 128), F32)

        def mix(x, ctx, first, fuse_h=False):
            if first:
                wait(g_g)
                start(g_o2)
                transpose_gu(0, wg)
                wait(g_u)
                start(g_d012)
                transpose_gu(1, wu)
                transpose_gu_last()
                onesL = jnp.ones((16, 128), BF)
                for n in range(2 * NFB + 1):
                    a = None
                    for mb in range(NMB):
                        a = _acc(a, _dot(onesL, _tile(guT_u, (n * NMB + mb) * 64))[0:8])
                    cs_scr[pl.ds(n * 8, 8), :] = a
                wait(g_o1)
                start(g_d34a)
            def flhs(h):
                hh, r = divmod(h, 16)
                return jnp.broadcast_to(ctx[hh][r:r + 1, :], (16, 128)).astype(BF)
            FV = opts.get('fv', ())
            acc = [None] * NMB
            vlo = [None] * NMB
            vhi = [None] * NMB

            mts = {}

            def f_group(h, k, dep):
                if h not in mts:
                    L = flhs(h)
                    mts[h] = pltpu.bitcast(jnp.concatenate([L] * 8, axis=0).T, U32)
                mk = mts[h][8 * k:8 * k + 8]
                if dep is not None:
                    mk = jnp.where(always, mk, pltpu.bitcast(dep, U32))
                mlo, mhi = unpack(mk)
                for mb in range(NMB):
                    wlo, whi = unpack(wo_u[pl.ds(mb * (SK // 2) + h * 64 + 8 * k, 8), :])
                    vlo[mb] = _acc(vlo[mb], wlo * mlo + whi * mhi)

            DEPD = opts.get('depd', 2)
            RHO = opts.get('rho', 1.0)

            def run_mixed(mh, vh):
                Lc = {}

                def f_tile(h, mb):
                    def fn():
                        if h not in Lc:
                            Lc[h] = flhs(h)
                        acc[mb] = _acc(acc[mb], _dot(Lc[h], _tile(wo_u, mb * (SK // 2) + h * 64))[0:8])
                        return acc[mb]
                    return fn

                def f_grp(h, k):
                    def fn(dep):
                        f_group(h, k, dep)
                        return vlo[NMB - 1]
                    return fn
                paced([f_tile(h, mb) for h in mh for mb in range(NMB)], [f_grp(h, k) for h in vh for k in range(8)], DEPD, RHO)
            run_mixed([h for h in range(NH1) if h not in FV], [h for h in range(NH1) if h in FV])
            if first:
                wait(g_o2)
                start(g_d34b)
            assert all(h < NH1 for h in FV)
            Ls = {h: flhs(h) for h in range(NH1, 32) if h not in FV}
            x1 = []
            for mb in range(NMB):
                for h in Ls:
                    acc[mb] = _acc(acc[mb], _dot(Ls[h], _tile(wo_u, mb * (SK // 2) + h * 64))[0:8])
                a = acc[mb]
                if FV:
                    a = a + jnp.sum(vlo[mb], axis=0, keepdims=True)
                x1.append(x[mb] + a)
            GV = tuple(opts.get('gv', ()))
            L = [_rep16(x1[b]) for b in range(NMB)]
            mean, inv = _stats(x1)
            xn1 = [(x1[b] - mean) * inv for b in range(NMB)]
            rr = xn1[0] * wr_rows[0]
            for b in range(1, NMB):
                rr = rr + xn1[b] * wr_rows[b]
            r = jnp.sum(rr, axis=1, keepdims=True)
            sig = 1.0 / (1.0 + jnp.exp(-r))

            def fin(a, n):
                return (a - mean * cs_scr[pl.ds(n * 8, 8), :]) * inv
            hs = [None] * (NFB + 1)
            sigt = [sig]
            accs = {}
            mfb = [fb for fb in range(NFB) if fb not in GV]
            mxu_fns = []

            HV = tuple(opts.get('hv', ()))
            mth = {}

            def g_tile(fb, which, mb):
                def fn():
                    o = _dot(L[mb], _tile(guT_u, gu_index(which, fb, mb) * 64))[0:8]
                    accs[fb, which] = _acc(accs.get((fb, which)), o)
                    res = o if opts.get('rawdep', 0) else accs[fb, which]
                    if which == 1 and mb == NMB - 1 and opts.get('early_hs', 1):
                        hs[fb] = silu(fin(accs[fb, 0], fb)) * fin(accs[fb, 1], NFB + fb)
                        if opts.get('sigtie', 0) and fb == mfb[opts.get('sigtie', 0)]:
                            hs[fb] = jnp.where(always, hs[fb], jnp.broadcast_to(sig, (8, 128)))
                        if fb in HV and not first:
                            mth[fb] = pltpu.bitcast(jnp.concatenate([_rep16(hs[fb])] * 8, axis=0).T, U32)
                    return res
                return fn
            for mb in range(NMB):
                for fb in mfb[:G1]:
                    for which in range(2):
                        mxu_fns.append(g_tile(fb, which, mb))
            for fb in mfb[G1:]:
                for which in range(2):
                    for mb in range(NMB):
                        mxu_fns.append(g_tile(fb, which, mb))
            vacc = {}
            mtg = {}

            def g_group(mb, k, which):
                def fn(dep):
                    if mb not in mtg:
                        mtg[mb] = pltpu.bitcast(jnp.concatenate([_rep16(x1[mb])] * 8, axis=0).T, U32)
                    mlo, mhi = unpack(tie(mtg[mb][8 * k:8 * k + 8], dep))
                    for fb in GV:
                        wlo, whi = unpack(guT_u[pl.ds(gu_index(which, fb, mb) * 64 + 8 * k, 8), :])
                        vacc[fb, which] = _acc(vacc.get((fb, which)), wlo * mlo + whi * mhi)
                    return vacc[GV[-1], which]
                return fn
            vpu_fns = [g_group(mb, k, which) for mb in range(NMB) for k in range(8) for which in range(2)] if GV else []
            lastacc = [None]

            def gl_tile(mb):
                def fn():
                    lastacc[0] = _acc(lastacc[0], _dot(L[mb], _tile(guT_u, (2 * NFB * NMB + mb) * 64))[0:8])
                    res = lastacc[0]
                    if mb == NMB - 1:
                        a = fin(res, 2 * NFB)
                        sw = pltpu.roll(a, 64, axis=1)
                        g = jnp.where(lane < 64, a, sw)
                        u = jnp.where(lane < 64, sw, a)
                        hs[NFB] = silu(g) * u
                    return res
                return fn
            mxu_fns += [gl_tile(mb) for mb in range(NMB)]

            def finish_mxu_blocks():
                for fb in mfb:
                    if hs[fb] is None:
                        hs[fb] = silu(fin(accs[fb, 0], fb)) * fin(accs[fb, 1], NFB + fb)

            def finish_vpu_blocks():
                for i, fb in enumerate(GV):
                    gu = []
                    for which in range(2):
                        raw = jnp.sum(vacc[fb, which], axis=0, keepdims=True)
                        gu.append(fin(raw, which * NFB + fb))
                    hs[fb] = silu(gu[0]) * gu[1]
            if not fuse_h:
                paced(mxu_fns, vpu_fns, opts.get('gdepd', 2), opts.get('grho', 1.0))
                finish_mxu_blocks()
                finish_vpu_blocks()
                return x1, xn1, sig, hs, mean
            h_mxu, h_vpu, h_done = h_streams(hs, mth, finish_mxu_blocks)
            ng = len(vpu_fns)

            def last_g_group(fn):
                def w(dep):
                    r = fn(dep)
                    finish_vpu_blocks()
                    return r
                return w
            if vpu_fns:
                vpu_fns[-1] = last_g_group(vpu_fns[-1])
            paced(mxu_fns + h_mxu, vpu_fns + h_vpu, opts.get('gdepd', 2), opts.get('grho', 1.0))
            return x1, xn1, sig, h_done(), None

        def h_last_lhs(hl):
            z = jnp.zeros_like(hl)
            ev = jnp.where(lane < 64, hl, z)
            od = jnp.where(lane < 64, z, hl)
            return _rep16(jnp.where(sub % 2 == 0, ev, od))

        def h_last_tile(L, mb, mb2):
            r0 = NFB * 64
            t = jnp.concatenate([wd_u[pl.ds(mb * (F // 2) + r0, 32), :], wd_u[pl.ds(mb2 * (F // 2) + r0, 32), :]], axis=0)
            return _dot(L, pltpu.bitcast(t, BF))[0:8]

        def h_streams(hs, mth, finish_mxu_blocks):
            GV = tuple(opts.get('gv', ()))
            HV = tuple(opts.get('hv', ()))
            acc = [None] * NMB
            order = [fb for fb in range(NFB) if fb not in GV] + [NFB] + list(GV)
            mxu_fns = []
            Lc = {}

            def h_tile(fb, mb):
                def fn():
                    if fb not in Lc:
                        finish_mxu_blocks()
                        Lc[fb] = _rep16(hs[fb])
                    o = _dot(Lc[fb], _tile(wd_u, mb * (F // 2) + fb * 64))[0:8]
                    acc[mb] = _acc(acc[mb], o)
                    return o if opts.get('rawdep', 0) else acc[mb]
                return fn

            def h_last(mb):
                def fn():
                    if NFB not in Lc:
                        Lc[NFB] = h_last_lhs(hs[NFB])
                    mb2 = min(mb + 1, NMB - 1)
                    o = h_last_tile(Lc[NFB], mb, mb2)
                    acc[mb] = acc[mb] + jnp.broadcast_to(o[0:1], (8, 128))
                    if mb2 != mb:
                        acc[mb2] = acc[mb2] + jnp.broadcast_to(o[1:2], (8, 128))
                    return acc[mb]
                return fn
            for fb in order:
                if fb in HV:
                    continue
                if fb == NFB:
                    mxu_fns += [h_last(mb) for mb in range(0, NMB, 2)]
                else:
                    mxu_fns += [h_tile(fb, mb) for mb in range(NMB)]
            vacc = [None] * NMB

            def h_group(fb, k):
                def fn(dep):
                    if fb not in mth:
                        finish_mxu_blocks()
                        mth[fb] = pltpu.bitcast(jnp.concatenate([_rep16(hs[fb])] * 8, axis=0).T, U32)
                    mlo, mhi = unpack(tie(mth[fb][8 * k:8 * k + 8], dep))
                    for mb in range(NMB):
                        wlo, whi = unpack(wd_u[pl.ds(mb * (F // 2) + fb * 64 + 8 * k, 8), :])
                        vacc[mb] = _acc(vacc[mb], wlo * mlo + whi * mhi)
                    return vacc[NMB - 1]
                return fn

            def done():
                if HV:
                    return [acc[mb] + jnp.sum(vacc[mb], axis=0, keepdims=True) for mb in range(NMB)]
                return acc
            return mxu_fns, [h_group(fb, k) for fb in HV for k in range(8)], done

        def next_layer_head(x1, xn1, sig, hs, first, mean1):
            Lh = [_rep16(hs[fb]) for fb in range(NFB)]
            Ll = h_last_lhs(hs[NFB])
            acc = [None] * NMB
            x2 = [None] * NMB
            q = [None, None]

            def hpart(fbs, mbs):
                for fb in fbs:
                    for mb in mbs:
                        acc[mb] = _acc(acc[mb], _dot(Lh[fb], _tile(wd_u, mb * (F // 2) + fb * 64))[0:8])

            def hlast(mb, mb2):
                o = h_last_tile(Ll, mb, mb2)
                acc[mb] = acc[mb] + jnp.broadcast_to(o[0:1], (8, 128))
                if mb2 != mb:
                    acc[mb2] = acc[mb2] + jnp.broadcast_to(o[1:2], (8, 128))

            NDEF = opts.get('ndef', 8)
            ds = {}

            def finish_x(mb):
                x2[mb] = x1[mb] + xn1[mb] + acc[mb] * sig
                ds[mb] = dup_bits(x2[mb])

            def ablock(mb, rs, hhs=(0, 1)):
                for r in rs:
                    l0 = xlhs(ds[mb], r, XQ)
                    for hh in hhs:
                        q[hh] = _acc(q[hh], _dot(l0, xtile(wq_u, 16 * mb + r, hh)))

            if first:
                wait(g_d012)
            hpart(range(NFB), (0, 1))
            hlast(0, 1)
            hpart(range(NFB), (2,))
            hlast(2, 2)
            finish_x(0)
            finish_x(1)
            ablock(0, range(16))
            finish_x(2)
            ablock(1, range(16))
            NCOV = opts.get('ncov', 8)
            ablock(2, range(16 - NCOV))
            if first:
                wait(g_d34a)
            hpart(range(FS34), (3, 4))
            if first:
                wait(g_d34b)
            if first and opts.get('stop', 0):
                return x2[:3] + [acc[3], acc[4]], q, [], [], {}, None
            mb = NMB - 1
            lcache = {}
            seg1 = [lambda fb=fb: hpart([fb], (3, 4)) for fb in range(FS34, NFB)]
            seg1.append(lambda: hlast(3, 4))

            def a_tile(blk, r, hh):
                def fn():
                    if not opts.get('lcache', 0) or (blk, r) not in lcache:
                        lcache[blk, r] = xlhs(ds[blk], r, XQ)
                        if blk == NMB - 1 and hh == 0 and r == opts.get('sttie', -1):
                            inv_b = jnp.broadcast_to(st[0][1], (8, 128))
                            lcache[blk, r] = pltpu.bitcast(tie(pltpu.bitcast(lcache[blk, r], U32), inv_b), BF)
                    o = _dot(lcache[blk, r], xtile(wq_u, 16 * blk + r, hh))
                    q[hh] = _acc(q[hh], o)
                    return o[0:8]
                return fn
            for r in range(16 - NCOV, 16):
                seg1 += [a_tile(2, r, 0), a_tile(2, r, 1)]
            st = []

            def fx():
                finish_x(3)
                finish_x(4)
                if opts.get('stshift', 1):
                    st.append(_stats_shift(x2, mean1))
                else:
                    st.append(_stats(x2))
                return a_tile(3, 0, 0)()
            seg1.append(fx)
            seg1 += [a_tile(3, r, 0) for r in range(1, 16)]
            H1A = opts.get('h1a', 0)
            seg1 += [a_tile(3, r, 1) for r in range(H1A)]
            seg1 += [a_tile(4, r, 0) for r in range(16)]
            vq = {}
            for fn in seg1:
                fn()
            tail = [a_tile(3, r, 1) for r in range(H1A, 16)] + [a_tile(4, r, 1) for r in range(16)]
            vtail = []
            if opts.get('stop', 0):
                for fn in tail:
                    fn()
            return x2, q, tail, vtail, vq, st[0]

        wait(g_q)
        start(g_uv)
        xrow = xb[0].astype(F32)
        x = [jnp.broadcast_to(xrow[:, b * 128:(b + 1) * 128], (8, 128)) for b in range(NMB)]
        wrf = wrb[...].astype(F32)
        wr_rows = [jnp.broadcast_to(wrf[b:b + 1, :], (8, 128)) for b in range(NMB)]
        always = (pltpu.bitcast(wr_rows[0], U32) | np.uint32(1)) != np.uint32(0)
        csq = colsum_q()
        q = [None, None]
        for mb in range(NMB):
            d = dup_bits(x[mb])
            xblock([d, d], wq_u, mb, q, mask=XQ)

        def make_finish(x, vq=None, st=None):
            mean, inv = _stats(x) if st is None else st
            def fin_q(raw, cs, hh):
                if vq and hh == 1:
                    raw = raw + jnp.concatenate([vq['e'], vq['o']], axis=0)
                return (raw - mean[0:1] * cs) * inv[0:1]
            return fin_q
        wait(g_uk)
        start(g_g)
        relayout_uk()
        ctx = attention(q, make_finish(x), csq, True)
        x1, xn1, sig, hs, mean1 = mix(x, ctx, True)
        for it in range(1 + extra):
            x, q, tail, vtail, vq, st2 = next_layer_head(x1, xn1, sig, hs, it == 0, mean1)
            if opts.get('stop', 0):
                out = jnp.concatenate([xb_[0:1] + q[0][0:1] + q[1][0:1] for xb_ in x], axis=1)
                o_ref[...] = out.astype(BF).reshape(1, 1, M)
                return
            ctx = attention(q, make_finish(x, vq, st2), csq, False, tail, vtail)
            if it < extra:
                x1, xn1, sig, hs, mean1 = mix(x, ctx, False)
            else:
                x1, xn1, sig, acc, _ = mix(x, ctx, False, fuse_h=True)
        xo = [x1[b] + xn1[b] + acc[b] * sig for b in range(NMB)]
        out = jnp.concatenate([xb_[0:1] for xb_ in xo], axis=1)
        o_ref[...] = out.astype(BF).reshape(1, 1, M)

    scratch = [
        pltpu.VMEM((1, 1, M), BF),
        pltpu.VMEM((NMB, 128), BF),
        pltpu.VMEM((M * H, D), BF),
        pltpu.VMEM((DC * H, D), BF),
        pltpu.VMEM((DC * H, D), BF),
        pltpu.VMEM((NCB * SK, 128), BF),
        pltpu.VMEM((NCB * SK, 128), BF),
        pltpu.VMEM((DC * H, D), BF),
        pltpu.VMEM((NMB * SK, 128), BF),
        pltpu.VMEM((F, M), BF),
        pltpu.VMEM((F, M), BF),
        pltpu.VMEM(((2 * NFB * NMB + NMB) * 128, 128), BF),
        pltpu.VMEM((NMB * F, 128), BF),
        pltpu.VMEM((H, SK), F32),
        pltpu.VMEM(((2 * NFB + 1) * 8, 128), F32),
        pltpu.VMEM((128, 128), BF),
        pltpu.SemaphoreType.DMA((3,)),
    ]

    def fn(A_x, A_c_kv, A_w_q, A_w_uk, A_w_uv, A_w_o, B_x, B_w_r, B_w_gate, B_w_up, B_w_down):
        return pl.pallas_call(
            kernel,
            out_shape=jax.ShapeDtypeStruct((1, 1, M), BF),
            in_specs=[pl.BlockSpec(memory_space=pltpu.HBM)] * 10,
            out_specs=pl.BlockSpec(memory_space=pltpu.VMEM),
            scratch_shapes=scratch,
            compiler_params=pltpu.CompilerParams(vmem_limit_bytes=100 * 1024 * 1024, flags=opts.get('flags', None)),
        )(A_x, B_w_r.reshape(NMB, 128), A_w_q.reshape(M * H, D), A_w_uk.reshape(DC * H, D),
          A_c_kv.reshape(SK, DC), A_w_uv.reshape(DC * H, D), A_w_o.reshape(H * D, M),
          B_w_gate.T, B_w_up.T, B_w_down)
    return fn


@jax.jit
def pallas_interleave_layers__compressed_kv_cla__moe_arch_mod__decode_kernel(
    A_x: jax.Array,
    A_c_kv: jax.Array,
    A_w_q: jax.Array,
    A_w_uk: jax.Array,
    A_w_uv: jax.Array,
    A_w_o: jax.Array,
    B_x: jax.Array,
    B_w_r: jax.Array,
    B_w_gate: jax.Array,
    B_w_up: jax.Array,
    B_w_down: jax.Array,
):
    fn = build({'ndef':16,'fs4':0,'nh1':28,'fv':(1,3,5,7,9,11,13,15,17,19),'gv':(9,10,11,12),'hv':(0,1,2),'depd':1,'grho':1.1,'g1':3,'sigtie':5,'nb2':12,'bv':(5,6,7),'bahead':0,'bskip':24,'av':0,'sttie':8,'bdepd':4,'wo_rc':16,'rs34':9,'brho':1.15})
    return fn(A_x, A_c_kv, A_w_q, A_w_uk, A_w_uv, A_w_o, B_x, B_w_r, B_w_gate, B_w_up, B_w_down)
```

```python
import functools
import contextlib
import numpy as np
import jax
import jax.numpy as jnp
from jax import lax
import jax.experimental.pallas as pl
import jax.experimental.pallas.tpu as pltpu

M, H, D, DC, SK, F = 640, 32, 128, 512, 4096, 1728
NMB = M // 128
NCB = DC // 128
NKB = SK // 128
NFB = F // 128
FREM = F - NFB * 128
LOG2E = 1.4426950408889634
EPS = 1e-5
BF = jnp.bfloat16
F32 = jnp.float32
U32 = jnp.uint32


def _dot(a, b):
    return jnp.dot(a, b, preferred_element_type=F32)


def _tile(ref_u32, r0):
    return pltpu.bitcast(ref_u32[pl.ds(r0, 64), :], BF)


def _iota(shape, ax):
    return lax.broadcasted_iota(jnp.int32, shape, ax)


def _pack_rows(v):
    return pltpu.bitcast(v.astype(BF), U32)


def _stats(x):
    s = x[0]
    for b in range(1, NMB):
        s = s + x[b]
    mean = jnp.sum(s, axis=1, keepdims=True) * (1.0 / M)
    xc = [xb - mean for xb in x]
    v = xc[0] * xc[0]
    for b in range(1, NMB):
        v = v + xc[b] * xc[b]
    var = jnp.sum(v, axis=1, keepdims=True) * (1.0 / M)
    return mean, lax.rsqrt(var + EPS)


def _stats_shift(x, shift):
    d = [xb - shift for xb in x]
    s1 = d[0]
    s2 = d[0] * d[0]
    for b in range(1, NMB):
        s1 = s1 + d[b]
        s2 = s2 + d[b] * d[b]
    m1 = jnp.sum(s1, axis=1, keepdims=True) * (1.0 / M)
    m2 = jnp.sum(s2, axis=1, keepdims=True) * (1.0 / M)
    var = jnp.maximum(m2 - m1 * m1, 0.0)
    return shift + m1, lax.rsqrt(var + EPS)


def _rep16(v):
    return jnp.concatenate([v, v], axis=0).astype(BF)


def unpack(w):
    lo = pltpu.bitcast(w << 16, F32)
    hi = pltpu.bitcast(w & np.uint32(0xFFFF0000), F32)
    return lo, hi


def _acc(a, o):
    return o if a is None else a + o


def build(opts=None):
    opts = dict(opts or {})
    WO_RC = opts.get('wo_rc', 8)
    WD_RC = opts.get('wd_rc', 12)
    WD_SPLIT = opts.get('wd_split', 9)
    NA = opts.get('na', 8)
    NB2 = opts.get('nb2', 8)
    G1 = opts.get('g1', 3)
    scoped = opts.get('scoped', False)
    extra = opts.get('extra', 0)

    def scope(name):
        if scoped:
            return jax.named_scope(name)
        import contextlib
        return contextlib.nullcontext()

    def kernel(x_hbm, wr_hbm, wq_hbm, wuk_hbm, ckv_hbm, wuv_hbm, wo_hbm, wg_hbm, wu_hbm, wd_hbm,
               o_ref,
               xb, wrb, wq, wuk, ukT, ckv, ckvT, wuv, wo, wg, wu, guT, wd, s_scr, cs_scr, mt_scr, sems):
        NSEM = opts.get('nsem', 3)

        def cp(src, dst):
            return (src, dst)
        g_q = [cp(wq_hbm, wq), cp(x_hbm, xb), cp(wr_hbm, wrb)]
        g_uk = [cp(wuk_hbm, wuk)]
        g_ckv = [cp(ckv_hbm.at[:, pl.ds(j * 128, 128)], ckv.at[pl.ds(j * SK, SK)]) for j in range(NCB)]
        g_uv = [cp(wuv_hbm, wuv)]
        g_g = [cp(wg_hbm, wg)]
        g_u = [cp(wu_hbm, wu)]
        NH1 = opts.get('nh1', 24)
        g_o1, g_o2 = [], []
        for r in range(WO_RC):
            n = SK // WO_RC
            for j in range(NMB):
                (g_o1 if r * n < NH1 * D else g_o2).append(
                    cp(wo_hbm.at[pl.ds(r * n, n), pl.ds(j * 128, 128)], wo.at[pl.ds(j * SK + r * n, n)]))
        nu = F // 64
        bounds = [(nu * j // WD_RC) * 64 for j in range(WD_RC + 1)]

        def slab(a, b, j):
            return cp(wd_hbm.at[pl.ds(a, b - a), pl.ds(j * 128, 128)], wd.at[pl.ds(j * F + a, b - a)])
        RS = opts.get('rs34', 9)
        FS34 = bounds[RS] // 128
        g_d012 = [slab(bounds[r], bounds[r + 1], j) for r in range(WD_RC) for j in (0, 1, 2)]
        g_d34a = [slab(bounds[r], bounds[r + 1], j) for r in range(RS) for j in (3, 4)]
        g_d34b = [slab(bounds[r], bounds[r + 1], j) for r in range(RS, WD_RC) for j in (3, 4)]
        groups = [g_q, g_uk, g_ckv, g_uv, g_g, g_u, g_o1, g_o2, g_d012, g_d34a, g_d34b]
        copies = [[pltpu.make_async_copy(a, b, sems.at[i % NSEM]) for a, b in g] for i, g in enumerate(groups)]
        nwaited = [0]

        def wait(grp):
            i = nwaited[0]
            assert grp is groups[i]
            with scope('wait%02d' % i):
                for c in copies[i]:
                    c.wait()
            if i + NSEM < len(groups):
                for c in copies[i + NSEM]:
                    c.start()
            nwaited[0] += 1

        for i in range(NSEM):
            for c in copies[i]:
                c.start()

        def write_out(val):
            if opts.get('manout', 0):
                xb[...] = val
                c = pltpu.make_async_copy(xb, o_ref, sems.at[0])
                c.start()
                c.wait()
            else:
                o_ref[...] = val

        if opts.get('dmaonly', 0):
            for g in groups:
                wait(g)
            write_out(xb[...])
            return
        lane = _iota((8, 128), 1)
        sub = _iota((8, 128), 0)
        h16 = lane % 16
        XM = jnp.where(h16 == 2 * sub, np.uint32(0x0000FFFF),
                       jnp.where(h16 == 2 * sub + 1, np.uint32(0xFFFF0000), np.uint32(0)))
        rlo, rhi = 2 * sub, 2 * sub + 1
        hlo = jnp.where(rlo < 8, 2 * rlo, 2 * (rlo - 8) + 1)
        hhi = jnp.where(rhi < 8, 2 * rhi, 2 * (rhi - 8) + 1)
        XQ = (jnp.where(h16 == hlo, np.uint32(0x0000FFFF), np.uint32(0))
              | jnp.where(h16 == hhi, np.uint32(0xFFFF0000), np.uint32(0)))
        idx16 = lane // 16
        PM = jnp.where(lane % 2 == 0, np.uint32(0x0000FFFF), np.uint32(0xFFFF0000))
        idx2 = lane // 2

        wq_u = wq.bitcast(U32)
        wuk_u = wuk.bitcast(U32)
        wuv_u = wuv.bitcast(U32)
        mt_u = mt_scr.bitcast(U32)
        ukT_u = ukT.bitcast(U32)
        ckv_u = ckv.bitcast(U32)
        ckvT_u = ckvT.bitcast(U32)
        wo_u = wo.bitcast(U32)
        guT_u = guT.bitcast(U32)
        wd_u = wd.bitcast(U32)

        def xtile(w_u, g, hh):
            rows = [w_u[pl.ds((8 * g + j) * 16 + 8 * hh, 8), :] for j in range(8)]
            return pltpu.bitcast(jnp.concatenate(rows, axis=0), BF)

        def xlhs(src, r, mask=None):
            mask = XM if mask is None else mask
            return pltpu.bitcast(jnp.take_along_axis(src, idx16 + 8 * r, axis=1) & mask, BF)

        def xblock(srcs, w_u, blk, acc, hhs=(0, 1), mask=None):
            for r in range(16):
                l0 = None
                for hh in hhs:
                    if l0 is None or srcs[hh] is not srcs[hhs[0]]:
                        l0 = xlhs(srcs[hh], r, mask)
                    acc[hh] = _acc(acc[hh], _dot(l0, xtile(w_u, 16 * blk + r, hh)))

        def dup_bits(v):
            u = pltpu.bitcast(v.astype(BF).astype(F32), U32)
            return u | (u >> 16)

        def colsum_q():
            if opts.get('no_cs', 0): return [jnp.zeros((16,128),F32)]*2
            l0 = pltpu.bitcast(XQ & np.uint32(0x3F803F80), BF)
            acc = [None, None]
            for g in range(M // 8):
                for hh in range(2):
                    acc[hh] = _acc(acc[hh], _dot(l0, xtile(wq_u, g, hh)))
            return acc

        def relayout_uk():
            if opts.get('no_uk', 0): return
            for hp in range(16):
                for cb in range(NCB):
                    s = wuk_u[pl.ds(128 * cb * 16 + hp, 128, stride=16), :]
                    ukT[pl.ds((hp * NCB + cb) * 256, 256), :] = pltpu.bitcast(s.T, BF)

        def transpose_ckv():
            if opts.get('no_ckv', 0): return
            for cb in range(NCB):
                for kb in range(NKB):
                    t = ckv[pl.ds(cb * SK + kb * 128, 128), :]
                    ckvT[pl.ds((cb * NKB + kb) * 128, 128), :] = t.T

        def gu_index(which, fb, mb):
            return (which * NFB + fb) * NMB + mb

        def transpose_gu(which, src):
            if opts.get('no_gu', 0): return
            for fb in range(NFB):
                for mb in range(NMB):
                    t = src[pl.ds(fb * 128, 128), pl.ds(mb * 128, 128)]
                    guT[pl.ds(gu_index(which, fb, mb) * 128, 128), :] = t.T

        def transpose_gu_last():
            for mb in range(NMB):
                t = jnp.concatenate([wg[pl.ds(NFB * 128, FREM), pl.ds(mb * 128, 128)],
                                     wu[pl.ds(NFB * 128, FREM), pl.ds(mb * 128, 128)]], axis=0)
                guT[pl.ds((2 * NFB * NMB + mb) * 128, 128), :] = t.T

        def b_block(L, hh, cb):
            acc = None
            for hp8 in range(8):
                hp = hh * 8 + hp8
                for kh in range(2):
                    Lm = pltpu.bitcast(jnp.where(sub == hp8, L[kh], np.uint32(0)), BF)
                    acc = _acc(acc, _dot(Lm, _tile(ukT_u, (hp * NCB + cb) * 128 + 64 * kh)))
            return acc

        def b_lhs(qh):
            qp = _pack_rows(qh)
            return [jnp.take_along_axis(qp, idx2 + 64 * kh, axis=1) & PM for kh in range(2)]

        CEXP = (D ** -0.5) * LOG2E

        def sblk(kb):
            return s_scr.at[:, kb * 128:(kb + 1) * 128]

        def attention(q_raw, finish_q, csq, first, pre_fns=(), pre_v=()):
            BV = tuple(opts.get('bv', ()))
            qa = [[None] * NCB for _ in range(2)]
            qps = {}

            def get_qp(hh):
                if hh not in qps:
                    qf = finish_q(q_raw[hh], csq[hh], hh)
                    qps[hh] = pltpu.bitcast(pltpu.pack_elementwise([qf[0:8], qf[8:16]], packed_dtype=BF), U32)
                return qps[hh]
            Lb = {}

            def b_tile(hh, cb, hp8, kh):
                def fn():
                    if hh not in Lb:
                        qp = get_qp(hh)
                        Lb[hh] = [jnp.take_along_axis(qp, idx2 + 64 * k2, axis=1) & PM for k2 in range(2)]
                    Lm = pltpu.bitcast(jnp.where(sub == hp8, Lb[hh][kh], np.uint32(0)), BF)
                    o = _dot(Lm, _tile(ukT_u, ((hh * 8 + hp8) * NCB + cb) * 128 + 64 * kh))
                    qa[hh][cb] = _acc(qa[hh][cb], o)
                    return o[0:8]
                return fn

            def b_fns(hh, cb):
                return [b_tile(hh, cb, hp8, kh) for hp8 in range(8) if (hh * 8 + hp8) not in BV for kh in range(2)]
            mtb = {}
            blo, bhi = {}, {}

            def mk_mtb(hp):
                if hp not in mtb:
                    qp = get_qp(hp // 8)
                    mtb[hp] = jnp.broadcast_to(qp[hp % 8:hp % 8 + 1, :], (128, 128)).T

            def b_group(hp, k):
                def fn(dep):
                    mk_mtb(hp)
                    i = BV.index(hp)
                    for ahead in range(1, opts.get('bahead', 0) + 1):
                        if i + ahead < len(BV):
                            mk_mtb(BV[i + ahead])
                    mlo, mhi = unpack(tie(mtb[hp][8 * k:8 * k + 8], dep))
                    for cb in range(NCB):
                        wlo, whi = unpack(ukT_u[pl.ds((hp * NCB + cb) * 128 + 8 * k, 8), :])
                        blo[hp, cb] = _acc(blo.get((hp, cb)), wlo * mlo)
                        bhi[hp, cb] = _acc(bhi.get((hp, cb)), whi * mhi)
                    return blo[hp, NCB - 1]
                return fn
            if BV:
                mk_mtb(BV[0])
                if len(BV) > 1 and opts.get('bahead', 0):
                    mk_mtb(BV[1])
            mfns = list(pre_fns)
            for cb in range(NCB):
                mfns += b_fns(0, cb)
            for cb in range(NCB - 1):
                mfns += b_fns(1, cb)
            paced(mfns, list(pre_v) + [b_group(hp, k) for hp in BV for k in range(16)], opts.get('bdepd', 2), opts.get('brho', 1.0), opts.get('bskip', 0))
            for hp in BV:
                hh, hp8 = divmod(hp, 8)
                v, r0 = hp8 // 4, 2 * (hp8 % 4)
                for cb in range(NCB):
                    lo, hi = blo[hp, cb], bhi[hp, cb]
                    u = jnp.where(sub % 2 == 0, lo + pltpu.roll(lo, 7, axis=0), hi + pltpu.roll(hi, 1, axis=0))
                    u = u + pltpu.roll(u, 2, axis=0)
                    u = u + pltpu.roll(u, 4, axis=0)
                    parts = [qa[hh][cb][0:8], qa[hh][cb][8:16]]
                    parts[v] = jnp.where((sub == r0) | (sub == r0 + 1), u, parts[v])
                    qa[hh][cb] = jnp.concatenate(parts, axis=0)

            def c_lhs(cb):
                return jnp.concatenate([qa[0][cb], qa[1][cb]], axis=0).astype(BF)
            if first:
                wait(g_ckv)
                transpose_ckv()
            lhs = [None] * NCB
            lhs[0] = c_lhs(0)
            for kb in range(NA):
                sblk(kb)[...] = _dot(lhs[0], _tile(ckvT_u, (0 * NKB + kb) * 64))
            for fn in b_fns(1, NCB - 1):
                fn()
            mx = None
            for cb in range(1, NCB):
                lhs[cb] = c_lhs(cb)
                for kb in range(NA):
                    s = sblk(kb)[...] + _dot(lhs[cb], _tile(ckvT_u, (cb * NKB + kb) * 64))
                    sblk(kb)[...] = s
                    if cb == NCB - 1:
                        mx = s if mx is None else jnp.maximum(mx, s)
            mA = jnp.max(mx, axis=1, keepdims=True)
            for kb in range(NA, NKB):
                s = None
                for cb in range(NCB):
                    s = _acc(s, _dot(lhs[cb], _tile(ckvT_u, (cb * NKB + kb) * 64)))
                sblk(kb)[...] = s
                mx = jnp.maximum(mx, s)
            mB = jnp.max(mx, axis=1, keepdims=True)
            acc = [None] * NCB
            l = None
            for kb in range(NA):
                p = jnp.exp2((sblk(kb)[...] - mA) * CEXP)
                l = _acc(l, p)
                pb = p.astype(BF)
                for cb in range(NCB):
                    acc[cb] = _acc(acc[cb], _dot(pb, _tile(ckv_u, cb * (SK // 2) + kb * 64)))
            alpha = jnp.exp2((mA - mB) * CEXP)
            acc = [a * alpha for a in acc]
            l = l * alpha
            for kb in range(NA, NKB - NB2):
                p = jnp.exp2((sblk(kb)[...] - mB) * CEXP)
                l = l + p
                pb = p.astype(BF)
                for cb in range(NCB):
                    acc[cb] = acc[cb] + _dot(pb, _tile(ckv_u, cb * (SK // 2) + kb * 64))
            pbs = []
            for kb in range(NKB - NB2, NKB):
                p = jnp.exp2((sblk(kb)[...] - mB) * CEXP)
                l = l + p
                pbs.append(p.astype(BF))
            linv = 1.0 / jnp.sum(l, axis=1, keepdims=True)
            srcs = []
            for cb in range(NCB):
                for i, kb in enumerate(range(NKB - NB2, NKB)):
                    acc[cb] = acc[cb] + _dot(pbs[i], _tile(ckv_u, cb * (SK // 2) + kb * 64))
                cc = acc[cb] * linv
                srcs.append([_pack_rows(cc[0:16]), _pack_rows(cc[16:32])])
            if first:
                wait(g_uv)
            ctx = [None, None]
            e1 = []
            if first or not opts.get('ehalf', 0):
                for cb in range(NCB - 1):
                    xblock(srcs[cb], wuv_u, cb, ctx)
                xblock(srcs[NCB - 1], wuv_u, NCB - 1, ctx, hhs=(0,))
                xblock(srcs[NCB - 1], wuv_u, NCB - 1, ctx, hhs=(1,))
            else:
                for cb in range(NCB):
                    xblock(srcs[cb], wuv_u, cb, ctx, hhs=(0,))

                def e_tile(cb, r):
                    def fn():
                        o = _dot(xlhs(srcs[cb][1], r), xtile(wuv_u, 16 * cb + r, 1))
                        ctx[1] = _acc(ctx[1], o)
                        return o[0:8]
                    return fn
                e1 = [e_tile(cb, r) for cb in range(NCB) for r in range(16)]
            ctx.append(e1)
            return ctx

        def paced(mxu_fns, vpu_fns, depd, rho_scale=1.0, skip=0):
            rho = len(vpu_fns) / max(1, len(mxu_fns) - skip) * rho_scale
            SELF = opts.get('self', 0)
            res = []
            vres = []
            j = 0

            def run_v(t):
                if SELF:
                    dep = vres[j - SELF] if j >= SELF else None
                else:
                    dep = res[max(t - depd, 0)] if depd >= 0 else None
                vres.append(vpu_fns[j](dep))
            for t, fn in enumerate(mxu_fns):
                res.append(fn())
                while j < len(vpu_fns) and j < rho * (t + 1 - skip):
                    run_v(t)
                    j += 1
            while j < len(vpu_fns):
                run_v(len(mxu_fns) - 1)
                j += 1

        def tie(v, dep):
            if dep is None:
                return v
            return jnp.where(always, v, pltpu.bitcast(dep, U32))

        def silu(g):
            return g / (1.0 + jnp.exp(-g))

        ones8 = jnp.ones((8, 128), F32)

        def mix(x, ctx, first, fuse_h=False):
            if first:
                wait(g_g)
                transpose_gu(0, wg)
                wait(g_u)
                transpose_gu(1, wu)
                transpose_gu_last()
                onesL = jnp.ones((16, 128), BF)
                for n in range(2 * NFB + 1):
                    a = None
                    for mb in range(NMB):
                        a = _acc(a, _dot(onesL, _tile(guT_u, (n * NMB + mb) * 64))[0:8])
                    cs_scr[pl.ds(n * 8, 8), :] = a
                wait(g_o1)
            def flhs(h):
                hh, r = divmod(h, 16)
                return jnp.broadcast_to(ctx[hh][r:r + 1, :], (16, 128)).astype(BF)
            FV = opts.get('fv', ())
            acc = [None] * NMB
            vlo = [None] * NMB
            vhi = [None] * NMB

            mts = {}

            def f_group(h, k, dep):
                if h not in mts:
                    L = flhs(h)
                    mts[h] = pltpu.bitcast(jnp.concatenate([L] * 8, axis=0).T, U32)
                mk = mts[h][8 * k:8 * k + 8]
                if dep is not None:
                    mk = jnp.where(always, mk, pltpu.bitcast(dep, U32))
                mlo, mhi = unpack(mk)
                for mb in range(NMB):
                    wlo, whi = unpack(wo_u[pl.ds(mb * (SK // 2) + h * 64 + 8 * k, 8), :])
                    vlo[mb] = _acc(vlo[mb], wlo * mlo + whi * mhi)

            DEPD = opts.get('depd', 2)
            RHO = opts.get('rho', 1.0)

            def run_mixed(mh, vh):
                Lc = {}

                def f_tile(h, mb):
                    def fn():
                        if h not in Lc:
                            Lc[h] = flhs(h)
                        acc[mb] = _acc(acc[mb], _dot(Lc[h], _tile(wo_u, mb * (SK // 2) + h * 64))[0:8])
                        return acc[mb]
                    return fn

                def f_grp(h, k):
                    def fn(dep):
                        f_group(h, k, dep)
                        return vlo[NMB - 1]
                    return fn
                paced(list(ctx[2]) + [f_tile(h, mb) for h in mh for mb in range(NMB)], [f_grp(h, k) for h in vh for k in range(8)], DEPD, RHO, opts.get('fskip', 0) if ctx[2] else 0)
            run_mixed([h for h in range(NH1) if h not in FV], [h for h in range(NH1) if h in FV])
            if first:
                wait(g_o2)
            assert all(h < NH1 for h in FV)
            Ls = {h: flhs(h) for h in range(NH1, 32) if h not in FV}
            x1 = []
            for mb in range(NMB):
                for h in Ls:
                    acc[mb] = _acc(acc[mb], _dot(Ls[h], _tile(wo_u, mb * (SK // 2) + h * 64))[0:8])
                a = acc[mb]
                if FV:
                    a = a + jnp.sum(vlo[mb], axis=0, keepdims=True)
                x1.append(x[mb] + a)
            GV = tuple(opts.get('gv', ()))
            L = [_rep16(x1[b]) for b in range(NMB)]
            mean, inv = _stats(x1)
            xn1 = [(x1[b] - mean) * inv for b in range(NMB)]
            rr = xn1[0] * wr_rows[0]
            for b in range(1, NMB):
                rr = rr + xn1[b] * wr_rows[b]
            r = jnp.sum(rr, axis=1, keepdims=True)
            sig = 1.0 / (1.0 + jnp.exp(-r))

            def fin(a, n):
                return (a - mean * cs_scr[pl.ds(n * 8, 8), :]) * inv
            hs = [None] * (NFB + 1)
            sigt = [sig]
            accs = {}
            ndone = {}
            mfb = [fb for fb in range(NFB) if fb not in GV]
            mxu_fns = []

            HV = tuple(opts.get('hv', ()))
            mth = {}

            def g_tile(fb, which, mb):
                def fn():
                    o = _dot(L[mb], _tile(guT_u, gu_index(which, fb, mb) * 64))[0:8]
                    ndone[fb] = ndone.get(fb, 0) + 1
                    accs[fb, which] = _acc(accs.get((fb, which)), o)
                    res = o if opts.get('rawdep', 0) else accs[fb, which]
                    if which == 1 and mb == NMB - 1 and opts.get('early_hs', 1):
                        hs[fb] = silu(fin(accs[fb, 0], fb)) * fin(accs[fb, 1], NFB + fb)
                        if opts.get('sigtie', 0) and fb == mfb[opts.get('sigtie', 0)]:
                            hs[fb] = jnp.where(always, hs[fb], jnp.broadcast_to(sig, (8, 128)))
                        if fb in HV and not first:
                            mth[fb] = pltpu.bitcast(jnp.concatenate([_rep16(hs[fb])] * 8, axis=0).T, U32)
                    return res
                return fn
            for mb in range(NMB):
                for fb in mfb[:G1]:
                    for which in range(2):
                        mxu_fns.append(g_tile(fb, which, mb))
            for fb in mfb[G1:]:
                for which in range(2):
                    for mb in range(NMB):
                        mxu_fns.append(g_tile(fb, which, mb))
            vacc = {}
            mtg = {}

            def g_group(mb, k, which):
                def fn(dep):
                    if mb not in mtg:
                        mtg[mb] = pltpu.bitcast(jnp.concatenate([_rep16(x1[mb])] * 8, axis=0).T, U32)
                    mlo, mhi = unpack(tie(mtg[mb][8 * k:8 * k + 8], dep))
                    for fb in GV:
                        wlo, whi = unpack(guT_u[pl.ds(gu_index(which, fb, mb) * 64 + 8 * k, 8), :])
                        vacc[fb, which] = _acc(vacc.get((fb, which)), wlo * mlo + whi * mhi)
                    return vacc[GV[-1], which]
                return fn
            vpu_fns = [g_group(mb, k, which) for mb in range(NMB) for k in range(8) for which in range(2)] if GV else []
            lastacc = [None]

            def gl_tile(mb):
                def fn():
                    lastacc[0] = _acc(lastacc[0], _dot(L[mb], _tile(guT_u, (2 * NFB * NMB + mb) * 64))[0:8])
                    res = lastacc[0]
                    if mb == NMB - 1:
                        a = fin(res, 2 * NFB)
                        sw = pltpu.roll(a, 64, axis=1)
                        g = jnp.where(lane < 64, a, sw)
                        u = jnp.where(lane < 64, sw, a)
                        hs[NFB] = silu(g) * u
                    return res
                return fn
            mxu_fns += [gl_tile(mb) for mb in range(NMB)]

            def finish_mxu_blocks(only=None):
                for fb in (mfb if only is None else [only]):
                    if hs[fb] is None:
                        assert ndone[fb] == 2 * NMB
                        hs[fb] = silu(fin(accs[fb, 0], fb)) * fin(accs[fb, 1], NFB + fb)

            def finish_vpu_blocks():
                for i, fb in enumerate(GV):
                    gu = []
                    for which in range(2):
                        raw = jnp.sum(vacc[fb, which], axis=0, keepdims=True)
                        gu.append(fin(raw, which * NFB + fb))
                    hs[fb] = silu(gu[0]) * gu[1]
            if not fuse_h:
                paced(mxu_fns, vpu_fns, opts.get('gdepd', 2), opts.get('grho', 1.0))
                finish_mxu_blocks()
                finish_vpu_blocks()
                return x1, xn1, sig, hs, mean
            h_mxu, h_vpu, h_done = h_streams(hs, mth, finish_mxu_blocks)
            ng = len(vpu_fns)

            def last_g_group(fn):
                def w(dep):
                    r = fn(dep)
                    finish_vpu_blocks()
                    return r
                return w
            if vpu_fns:
                vpu_fns[-1] = last_g_group(vpu_fns[-1])
            paced(mxu_fns + h_mxu, vpu_fns + h_vpu, opts.get('gdepd', 2), opts.get('grho', 1.0))
            return x1, xn1, sig, h_done(), None

        def h_last_lhs(hl):
            z = jnp.zeros_like(hl)
            ev = jnp.where(lane < 64, hl, z)
            od = jnp.where(lane < 64, z, hl)
            return _rep16(jnp.where(sub % 2 == 0, ev, od))

        def h_last_tile(L, mb, mb2):
            r0 = NFB * 64
            t = jnp.concatenate([wd_u[pl.ds(mb * (F // 2) + r0, 32), :], wd_u[pl.ds(mb2 * (F // 2) + r0, 32), :]], axis=0)
            return _dot(L, pltpu.bitcast(t, BF))[0:8]

        def h_streams(hs, mth, finish_mxu_blocks):
            GV = tuple(opts.get('gv', ()))
            HV = tuple(opts.get('hv', ()))
            acc = [None] * NMB
            order = [fb for fb in range(NFB) if fb not in GV] + [NFB] + list(GV)
            mxu_fns = []
            Lc = {}

            def h_tile(fb, mb):
                def fn():
                    if fb not in Lc:
                        finish_mxu_blocks(fb if opts.get('lazyfin', 1) and fb not in GV else None)
                        Lc[fb] = _rep16(hs[fb])
                    o = _dot(Lc[fb], _tile(wd_u, mb * (F // 2) + fb * 64))[0:8]
                    acc[mb] = _acc(acc[mb], o)
                    return o if opts.get('rawdep', 0) else acc[mb]
                return fn

            def h_last(mb):
                def fn():
                    if NFB not in Lc:
                        Lc[NFB] = h_last_lhs(hs[NFB])
                    mb2 = min(mb + 1, NMB - 1)
                    o = h_last_tile(Lc[NFB], mb, mb2)
                    acc[mb] = acc[mb] + jnp.broadcast_to(o[0:1], (8, 128))
                    if mb2 != mb:
                        acc[mb2] = acc[mb2] + jnp.broadcast_to(o[1:2], (8, 128))
                    return acc[mb]
                return fn
            for fb in order:
                if fb in HV:
                    continue
                if fb == NFB:
                    mxu_fns += [h_last(mb) for mb in range(0, NMB, 2)]
                else:
                    mxu_fns += [h_tile(fb, mb) for mb in range(NMB)]
            vacc = [None] * NMB

            def h_group(fb, k):
                def fn(dep):
                    if fb not in mth:
                        finish_mxu_blocks(fb if opts.get('lazyfin', 1) else None)
                        mth[fb] = pltpu.bitcast(jnp.concatenate([_rep16(hs[fb])] * 8, axis=0).T, U32)
                    mlo, mhi = unpack(tie(mth[fb][8 * k:8 * k + 8], dep))
                    for mb in range(NMB):
                        wlo, whi = unpack(wd_u[pl.ds(mb * (F // 2) + fb * 64 + 8 * k, 8), :])
                        vacc[mb] = _acc(vacc[mb], wlo * mlo + whi * mhi)
                    return vacc[NMB - 1]
                return fn

            def done():
                if HV:
                    return [acc[mb] + jnp.sum(vacc[mb], axis=0, keepdims=True) for mb in range(NMB)]
                return acc
            return mxu_fns, [h_group(fb, k) for fb in HV for k in range(8)], done

        def next_layer_head(x1, xn1, sig, hs, first, mean1):
            Lh = [_rep16(hs[fb]) for fb in range(NFB)]
            Ll = h_last_lhs(hs[NFB])
            acc = [None] * NMB
            x2 = [None] * NMB
            q = [None, None]

            def hpart(fbs, mbs):
                for fb in fbs:
                    for mb in mbs:
                        acc[mb] = _acc(acc[mb], _dot(Lh[fb], _tile(wd_u, mb * (F // 2) + fb * 64))[0:8])

            def hlast(mb, mb2):
                o = h_last_tile(Ll, mb, mb2)
                acc[mb] = acc[mb] + jnp.broadcast_to(o[0:1], (8, 128))
                if mb2 != mb:
                    acc[mb2] = acc[mb2] + jnp.broadcast_to(o[1:2], (8, 128))

            NDEF = opts.get('ndef', 8)
            ds = {}

            def finish_x(mb):
                x2[mb] = x1[mb] + xn1[mb] + acc[mb] * sig
                ds[mb] = dup_bits(x2[mb])

            def ablock(mb, rs, hhs=(0, 1)):
                for r in rs:
                    l0 = xlhs(ds[mb], r, XQ)
                    for hh in hhs:
                        q[hh] = _acc(q[hh], _dot(l0, xtile(wq_u, 16 * mb + r, hh)))

            if first:
                wait(g_d012)
            hpart(range(NFB), (0, 1))
            hlast(0, 1)
            hpart(range(NFB), (2,))
            hlast(2, 2)
            finish_x(0)
            finish_x(1)
            ablock(0, range(16))
            finish_x(2)
            ablock(1, range(16))
            NCOV = opts.get('ncov', 8)
            ablock(2, range(16 - NCOV))
            if first:
                wait(g_d34a)
            hpart(range(FS34), (3, 4))
            if first:
                wait(g_d34b)
            if first and opts.get('stop', 0):
                return x2[:3] + [acc[3], acc[4]], q, [], [], {}, None
            mb = NMB - 1
            lcache = {}
            seg1 = [lambda fb=fb: hpart([fb], (3, 4)) for fb in range(FS34, NFB)]
            seg1.append(lambda: hlast(3, 4))

            def a_tile(blk, r, hh):
                def fn():
                    if not opts.get('lcache', 0) or (blk, r) not in lcache:
                        lcache[blk, r] = xlhs(ds[blk], r, XQ)
                        if blk == NMB - 1 and hh == 0 and r == opts.get('sttie', -1):
                            inv_b = jnp.broadcast_to(st[0][1], (8, 128))
                            lcache[blk, r] = pltpu.bitcast(tie(pltpu.bitcast(lcache[blk, r], U32), inv_b), BF)
                    o = _dot(lcache[blk, r], xtile(wq_u, 16 * blk + r, hh))
                    q[hh] = _acc(q[hh], o)
                    return o[0:8]
                return fn
            for r in range(16 - NCOV, 16):
                seg1 += [a_tile(2, r, 0), a_tile(2, r, 1)]
            st = []

            def fx():
                finish_x(3)
                finish_x(4)
                if opts.get('stshift', 1):
                    st.append(_stats_shift(x2, mean1))
                else:
                    st.append(_stats(x2))
                return a_tile(3, 0, 0)()
            seg1.append(fx)
            seg1 += [a_tile(3, r, 0) for r in range(1, 16)]
            H1A = opts.get('h1a', 0)
            seg1 += [a_tile(3, r, 1) for r in range(H1A)]
            seg1 += [a_tile(4, r, 0) for r in range(16)]
            vq = {}
            for fn in seg1:
                fn()
            tail = [a_tile(3, r, 1) for r in range(H1A, 16)] + [a_tile(4, r, 1) for r in range(16)]
            vtail = []
            if opts.get('stop', 0):
                for fn in tail:
                    fn()
            return x2, q, tail, vtail, vq, st[0]

        wait(g_q)
        xrow = xb[0].astype(F32)
        x = [jnp.broadcast_to(xrow[:, b * 128:(b + 1) * 128], (8, 128)) for b in range(NMB)]
        wrf = wrb[...].astype(F32)
        wr_rows = [jnp.broadcast_to(wrf[b:b + 1, :], (8, 128)) for b in range(NMB)]
        always = (pltpu.bitcast(wr_rows[0], U32) | np.uint32(1)) != np.uint32(0)
        csq = colsum_q()
        q = [None, None]
        for mb in range(NMB):
            d = dup_bits(x[mb])
            xblock([d, d], wq_u, mb, q, mask=XQ)

        def make_finish(x, vq=None, st=None):
            mean, inv = _stats(x) if st is None else st
            def fin_q(raw, cs, hh):
                if vq and hh == 1:
                    raw = raw + jnp.concatenate([vq['e'], vq['o']], axis=0)
                return (raw - mean[0:1] * cs) * inv[0:1]
            return fin_q
        wait(g_uk)
        relayout_uk()
        ctx = attention(q, make_finish(x), csq, True)
        x1, xn1, sig, hs, mean1 = mix(x, ctx, True)
        for it in range(1 + extra):
            x, q, tail, vtail, vq, st2 = next_layer_head(x1, xn1, sig, hs, it == 0, mean1)
            if opts.get('stop', 0):
                out = jnp.concatenate([xb_[0:1] + q[0][0:1] + q[1][0:1] for xb_ in x], axis=1)
                write_out(out.astype(BF).reshape(1, 1, M))
                return
            ctx = attention(q, make_finish(x, vq, st2), csq, False, tail, vtail)
            if it < extra:
                x1, xn1, sig, hs, mean1 = mix(x, ctx, False)
            else:
                x1, xn1, sig, acc, _ = mix(x, ctx, False, fuse_h=True)
        xo = [x1[b] + xn1[b] + acc[b] * sig for b in range(NMB)]
        out = jnp.concatenate([xb_[0:1] for xb_ in xo], axis=1)
        write_out(out.astype(BF).reshape(1, 1, M))

    scratch = [
        pltpu.VMEM((1, 1, M), BF),
        pltpu.VMEM((NMB, 128), BF),
        pltpu.VMEM((M * H, D), BF),
        pltpu.VMEM((DC * H, D), BF),
        pltpu.VMEM((DC * H, D), BF),
        pltpu.VMEM((NCB * SK, 128), BF),
        pltpu.VMEM((NCB * SK, 128), BF),
        pltpu.VMEM((DC * H, D), BF),
        pltpu.VMEM((NMB * SK, 128), BF),
        pltpu.VMEM((F, M), BF),
        pltpu.VMEM((F, M), BF),
        pltpu.VMEM(((2 * NFB * NMB + NMB) * 128, 128), BF),
        pltpu.VMEM((NMB * F, 128), BF),
        pltpu.VMEM((H, SK), F32),
        pltpu.VMEM(((2 * NFB + 1) * 8, 128), F32),
        pltpu.VMEM((128, 128), BF),
        pltpu.SemaphoreType.DMA((opts.get('nsem', 3),)),
    ]

    def fn(A_x, A_c_kv, A_w_q, A_w_uk, A_w_uv, A_w_o, B_x, B_w_r, B_w_gate, B_w_up, B_w_down):
        return pl.pallas_call(
            kernel,
            out_shape=jax.ShapeDtypeStruct((1, 1, M), BF),
            in_specs=[pl.BlockSpec(memory_space=pltpu.HBM)] * 10,
            out_specs=pl.BlockSpec(memory_space=pltpu.HBM if opts.get('manout', 0) else pltpu.VMEM),
            scratch_shapes=scratch,
            compiler_params=pltpu.CompilerParams(vmem_limit_bytes=100 * 1024 * 1024, flags=opts.get('flags', None)),
        )(A_x, B_w_r.reshape(NMB, 128), A_w_q.reshape(M * H, D), A_w_uk.reshape(DC * H, D),
          A_c_kv.reshape(SK, DC), A_w_uv.reshape(DC * H, D), A_w_o.reshape(H * D, M),
          B_w_gate.T, B_w_up.T, B_w_down)
    return fn


@jax.jit
def pallas_interleave_layers__compressed_kv_cla__moe_arch_mod__decode_kernel(
    A_x: jax.Array,
    A_c_kv: jax.Array,
    A_w_q: jax.Array,
    A_w_uk: jax.Array,
    A_w_uv: jax.Array,
    A_w_o: jax.Array,
    B_x: jax.Array,
    B_w_r: jax.Array,
    B_w_gate: jax.Array,
    B_w_up: jax.Array,
    B_w_down: jax.Array,
):
    fn = build({'ndef':16,'fs4':0,'nh1':28,'fv':(0,1,2,3,4,5,6,7,8,9,10,11),'gv':(9,10,11,12),'hv':(0,1,2),'depd':1,'grho':1.1,'g1':3,'sigtie':0,'nb2':12,'bv':(5,6,7),'bahead':0,'bskip':24,'av':0,'sttie':8,'bdepd':4,'wo_rc':16,'rs34':9,'brho':1.15,'early_hs':0,'ehalf':1,'fskip':40})
    return fn(A_x, A_c_kv, A_w_q, A_w_uk, A_w_uv, A_w_o, B_x, B_w_r, B_w_gate, B_w_up, B_w_down)
```

```python
import numpy as np
import jax
import jax.numpy as jnp
from jax import lax
import jax.experimental.pallas as pl
import jax.experimental.pallas.tpu as pltpu

M, H, D, DC, SK, F = 640, 32, 128, 512, 4096, 1728
NMB = M // 128
NCB = DC // 128
NKB = SK // 128
NFB = F // 128
FREM = F - NFB * 128
LOG2E = 1.4426950408889634
EPS = 1e-5
BF = jnp.bfloat16
F32 = jnp.float32
U32 = jnp.uint32

NSEM = 3
WO_RC = 16
WD_RC = 12
WD_RS = 9
NH1 = 28
NA = 8
NB2 = 12
G1 = 3
NCOV = 8
BV = (5, 6, 7)
FV = tuple(range(12))
GV = (9, 10, 11, 12)
HV = (0, 1, 2)


def _dot(a, b):
    return jnp.dot(a, b, preferred_element_type=F32)


def _tile(ref_u32, r0):
    return pltpu.bitcast(ref_u32[pl.ds(r0, 64), :], BF)


def _iota(shape, ax):
    return lax.broadcasted_iota(jnp.int32, shape, ax)


def _pack_rows(v):
    return pltpu.bitcast(v.astype(BF), U32)


def _stats(x):
    s = x[0]
    for b in range(1, NMB):
        s = s + x[b]
    mean = jnp.sum(s, axis=1, keepdims=True) * (1.0 / M)
    xc = [xb - mean for xb in x]
    v = xc[0] * xc[0]
    for b in range(1, NMB):
        v = v + xc[b] * xc[b]
    var = jnp.sum(v, axis=1, keepdims=True) * (1.0 / M)
    return mean, lax.rsqrt(var + EPS)


def _stats_shift(x, shift):
    d = [xb - shift for xb in x]
    s1 = d[0]
    s2 = d[0] * d[0]
    for b in range(1, NMB):
        s1 = s1 + d[b]
        s2 = s2 + d[b] * d[b]
    m1 = jnp.sum(s1, axis=1, keepdims=True) * (1.0 / M)
    m2 = jnp.sum(s2, axis=1, keepdims=True) * (1.0 / M)
    var = jnp.maximum(m2 - m1 * m1, 0.0)
    return shift + m1, lax.rsqrt(var + EPS)


def _rep16(v):
    return jnp.concatenate([v, v], axis=0).astype(BF)


def _unpack(w):
    return pltpu.bitcast(w << 16, F32), pltpu.bitcast(w & np.uint32(0xFFFF0000), F32)


def _acc(a, o):
    return o if a is None else a + o


def _silu(g):
    return g / (1.0 + jnp.exp(-g))


def _col_multipliers(row16):
    return pltpu.bitcast(jnp.concatenate([row16] * 8, axis=0).T, U32)


def _kernel(x_hbm, wr_hbm, wq_hbm, wuk_hbm, ckv_hbm, wuv_hbm, wo_hbm, wg_hbm, wu_hbm, wd_hbm,
            o_ref,
            xb, wrb, wq, wuk, ukT, ckv, ckvT, wuv, wo, wg, wu, guT, wd, s_scr, cs_scr, sems):
    g_q = [(wq_hbm, wq), (x_hbm, xb), (wr_hbm, wrb)]
    g_uk = [(wuk_hbm, wuk)]
    g_ckv = [(ckv_hbm.at[:, pl.ds(j * 128, 128)], ckv.at[pl.ds(j * SK, SK)]) for j in range(NCB)]
    g_uv = [(wuv_hbm, wuv)]
    g_g = [(wg_hbm, wg)]
    g_u = [(wu_hbm, wu)]
    g_o1, g_o2 = [], []
    n = SK // WO_RC
    for r in range(WO_RC):
        for j in range(NMB):
            (g_o1 if r * n < NH1 * D else g_o2).append(
                (wo_hbm.at[pl.ds(r * n, n), pl.ds(j * 128, 128)], wo.at[pl.ds(j * SK + r * n, n)]))
    bounds = [(F // 64 * j // WD_RC) * 64 for j in range(WD_RC + 1)]

    def slab(r, j):
        a, b = bounds[r], bounds[r + 1]
        return (wd_hbm.at[pl.ds(a, b - a), pl.ds(j * 128, 128)], wd.at[pl.ds(j * F + a, b - a)])
    FS34 = bounds[WD_RS] // 128
    g_d012 = [slab(r, j) for r in range(WD_RC) for j in (0, 1, 2)]
    g_d34a = [slab(r, j) for r in range(WD_RS) for j in (3, 4)]
    g_d34b = [slab(r, j) for r in range(WD_RS, WD_RC) for j in (3, 4)]
    groups = [g_q, g_uk, g_ckv, g_uv, g_g, g_u, g_o1, g_o2, g_d012, g_d34a, g_d34b]
    copies = [[pltpu.make_async_copy(a, b, sems.at[i % NSEM]) for a, b in g] for i, g in enumerate(groups)]
    nwaited = [0]

    def wait(grp):
        i = nwaited[0]
        assert grp is groups[i]
        for c in copies[i]:
            c.wait()
        if i + NSEM < len(groups):
            for c in copies[i + NSEM]:
                c.start()
        nwaited[0] += 1

    for i in range(NSEM):
        for c in copies[i]:
            c.start()

    lane = _iota((8, 128), 1)
    sub = _iota((8, 128), 0)
    h16 = lane % 16
    XM = jnp.where(h16 == 2 * sub, np.uint32(0x0000FFFF),
                   jnp.where(h16 == 2 * sub + 1, np.uint32(0xFFFF0000), np.uint32(0)))
    rlo, rhi = 2 * sub, 2 * sub + 1
    hlo = jnp.where(rlo < 8, 2 * rlo, 2 * (rlo - 8) + 1)
    hhi = jnp.where(rhi < 8, 2 * rhi, 2 * (rhi - 8) + 1)
    XQ = (jnp.where(h16 == hlo, np.uint32(0x0000FFFF), np.uint32(0))
          | jnp.where(h16 == hhi, np.uint32(0xFFFF0000), np.uint32(0)))
    idx16 = lane // 16
    PM = jnp.where(lane % 2 == 0, np.uint32(0x0000FFFF), np.uint32(0xFFFF0000))
    idx2 = lane // 2

    wq_u = wq.bitcast(U32)
    wuk_u = wuk.bitcast(U32)
    wuv_u = wuv.bitcast(U32)
    ukT_u = ukT.bitcast(U32)
    ckv_u = ckv.bitcast(U32)
    ckvT_u = ckvT.bitcast(U32)
    wo_u = wo.bitcast(U32)
    guT_u = guT.bitcast(U32)
    wd_u = wd.bitcast(U32)

    def tie(v, dep):
        return jnp.where(always, v, pltpu.bitcast(dep, U32))

    def paced(mxu_fns, vpu_fns, depd, rho_scale, skip):
        rho = len(vpu_fns) / (len(mxu_fns) - skip) * rho_scale
        res = []
        j = 0
        for t, fn in enumerate(mxu_fns):
            res.append(fn())
            while j < len(vpu_fns) and j < rho * (t + 1 - skip):
                vpu_fns[j](res[max(t - depd, 0)])
                j += 1
        while j < len(vpu_fns):
            vpu_fns[j](res[max(len(mxu_fns) - 1 - depd, 0)])
            j += 1

    def xtile(w_u, g, hh):
        rows = [w_u[pl.ds((8 * g + j) * 16 + 8 * hh, 8), :] for j in range(8)]
        return pltpu.bitcast(jnp.concatenate(rows, axis=0), BF)

    def xlhs(src, r, mask):
        return pltpu.bitcast(jnp.take_along_axis(src, idx16 + 8 * r, axis=1) & mask, BF)

    def xblock(srcs, w_u, blk, acc, mask, rs=range(16), hhs=(0, 1)):
        for r in rs:
            l0 = None
            for hh in hhs:
                if l0 is None or srcs[hh] is not srcs[hhs[0]]:
                    l0 = xlhs(srcs[hh], r, mask)
                acc[hh] = _acc(acc[hh], _dot(l0, xtile(w_u, 16 * blk + r, hh)))

    def dup_bits(v):
        u = pltpu.bitcast(v.astype(BF).astype(F32), U32)
        return u | (u >> 16)

    def colsum_q():
        l0 = pltpu.bitcast(XQ & np.uint32(0x3F803F80), BF)
        acc = [None, None]
        for g in range(M // 8):
            for hh in range(2):
                acc[hh] = _acc(acc[hh], _dot(l0, xtile(wq_u, g, hh)))
        return acc

    def relayout_uk():
        for hp in range(H // 2):
            for cb in range(NCB):
                s = wuk_u[pl.ds(128 * cb * 16 + hp, 128, stride=16), :]
                ukT[pl.ds((hp * NCB + cb) * 256, 256), :] = pltpu.bitcast(s.T, BF)

    def transpose_ckv():
        for cb in range(NCB):
            for kb in range(NKB):
                ckvT[pl.ds((cb * NKB + kb) * 128, 128), :] = ckv[pl.ds(cb * SK + kb * 128, 128), :].T

    def gu_index(which, fb, mb):
        return (which * NFB + fb) * NMB + mb

    def transpose_gu(which, src):
        for fb in range(NFB):
            for mb in range(NMB):
                t = src[pl.ds(fb * 128, 128), pl.ds(mb * 128, 128)]
                guT[pl.ds(gu_index(which, fb, mb) * 128, 128), :] = t.T

    def transpose_gu_last():
        for mb in range(NMB):
            t = jnp.concatenate([wg[pl.ds(NFB * 128, FREM), pl.ds(mb * 128, 128)],
                                 wu[pl.ds(NFB * 128, FREM), pl.ds(mb * 128, 128)]], axis=0)
            guT[pl.ds((2 * NFB * NMB + mb) * 128, 128), :] = t.T

    CEXP = (D ** -0.5) * LOG2E

    def sblk(kb):
        return s_scr.at[:, kb * 128:(kb + 1) * 128]

    def attention(q_raw, st, csq, first, pre_fns=()):
        mean, inv = st
        qa = [[None] * NCB for _ in range(2)]
        qps, Lb = {}, {}

        def get_qp(hh):
            if hh not in qps:
                qf = (q_raw[hh] - mean[0:1] * csq[hh]) * inv[0:1]
                qps[hh] = pltpu.bitcast(pltpu.pack_elementwise([qf[0:8], qf[8:16]], packed_dtype=BF), U32)
            return qps[hh]

        def b_tile(hh, cb, hp8, kh):
            def fn():
                if hh not in Lb:
                    qp = get_qp(hh)
                    Lb[hh] = [jnp.take_along_axis(qp, idx2 + 64 * k2, axis=1) & PM for k2 in range(2)]
                Lm = pltpu.bitcast(jnp.where(sub == hp8, Lb[hh][kh], np.uint32(0)), BF)
                o = _dot(Lm, _tile(ukT_u, ((hh * 8 + hp8) * NCB + cb) * 128 + 64 * kh))
                qa[hh][cb] = _acc(qa[hh][cb], o)
                return o[0:8]
            return fn

        def b_fns(hh, cb):
            return [b_tile(hh, cb, hp8, kh) for hp8 in range(8) if (hh * 8 + hp8) not in BV for kh in range(2)]
        mtb, blo, bhi = {}, {}, {}

        def mk_mtb(hp):
            if hp not in mtb:
                qp = get_qp(hp // 8)
                mtb[hp] = jnp.broadcast_to(qp[hp % 8:hp % 8 + 1, :], (128, 128)).T

        def b_group(hp, k):
            def fn(dep):
                mk_mtb(hp)
                mlo, mhi = _unpack(tie(mtb[hp][8 * k:8 * k + 8], dep))
                for cb in range(NCB):
                    wlo, whi = _unpack(ukT_u[pl.ds((hp * NCB + cb) * 128 + 8 * k, 8), :])
                    blo[hp, cb] = _acc(blo.get((hp, cb)), wlo * mlo)
                    bhi[hp, cb] = _acc(bhi.get((hp, cb)), whi * mhi)
            return fn
        mk_mtb(BV[0])
        mfns = list(pre_fns)
        for cb in range(NCB):
            mfns += b_fns(0, cb)
        for cb in range(NCB - 1):
            mfns += b_fns(1, cb)
        paced(mfns, [b_group(hp, k) for hp in BV for k in range(16)], 4, 1.15, 24)
        for hp in BV:
            hh, hp8 = divmod(hp, 8)
            v, r0 = hp8 // 4, 2 * (hp8 % 4)
            for cb in range(NCB):
                lo, hi = blo[hp, cb], bhi[hp, cb]
                u = jnp.where(sub % 2 == 0, lo + pltpu.roll(lo, 7, axis=0), hi + pltpu.roll(hi, 1, axis=0))
                u = u + pltpu.roll(u, 2, axis=0)
                u = u + pltpu.roll(u, 4, axis=0)
                parts = [qa[hh][cb][0:8], qa[hh][cb][8:16]]
                parts[v] = jnp.where((sub == r0) | (sub == r0 + 1), u, parts[v])
                qa[hh][cb] = jnp.concatenate(parts, axis=0)

        def c_lhs(cb):
            return jnp.concatenate([qa[0][cb], qa[1][cb]], axis=0).astype(BF)
        if first:
            wait(g_ckv)
            transpose_ckv()
        lhs = [None] * NCB
        lhs[0] = c_lhs(0)
        for kb in range(NA):
            sblk(kb)[...] = _dot(lhs[0], _tile(ckvT_u, kb * 64))
        for fn in b_fns(1, NCB - 1):
            fn()
        mx = None
        for cb in range(1, NCB):
            lhs[cb] = c_lhs(cb)
            for kb in range(NA):
                s = sblk(kb)[...] + _dot(lhs[cb], _tile(ckvT_u, (cb * NKB + kb) * 64))
                sblk(kb)[...] = s
                if cb == NCB - 1:
                    mx = s if mx is None else jnp.maximum(mx, s)
        mA = jnp.max(mx, axis=1, keepdims=True)
        for kb in range(NA, NKB):
            s = None
            for cb in range(NCB):
                s = _acc(s, _dot(lhs[cb], _tile(ckvT_u, (cb * NKB + kb) * 64)))
            sblk(kb)[...] = s
            mx = jnp.maximum(mx, s)
        mB = jnp.max(mx, axis=1, keepdims=True)
        acc = [None] * NCB
        l = None
        for kb in range(NA):
            p = jnp.exp2((sblk(kb)[...] - mA) * CEXP)
            l = _acc(l, p)
            pb = p.astype(BF)
            for cb in range(NCB):
                acc[cb] = _acc(acc[cb], _dot(pb, _tile(ckv_u, cb * (SK // 2) + kb * 64)))
        alpha = jnp.exp2((mA - mB) * CEXP)
        acc = [a * alpha for a in acc]
        l = l * alpha
        for kb in range(NA, NKB - NB2):
            p = jnp.exp2((sblk(kb)[...] - mB) * CEXP)
            l = l + p
            pb = p.astype(BF)
            for cb in range(NCB):
                acc[cb] = acc[cb] + _dot(pb, _tile(ckv_u, cb * (SK // 2) + kb * 64))
        pbs = []
        for kb in range(NKB - NB2, NKB):
            p = jnp.exp2((sblk(kb)[...] - mB) * CEXP)
            l = l + p
            pbs.append(p.astype(BF))
        linv = 1.0 / jnp.sum(l, axis=1, keepdims=True)
        srcs = []
        for cb in range(NCB):
            for i, kb in enumerate(range(NKB - NB2, NKB)):
                acc[cb] = acc[cb] + _dot(pbs[i], _tile(ckv_u, cb * (SK // 2) + kb * 64))
            cc = acc[cb] * linv
            srcs.append([_pack_rows(cc[0:16]), _pack_rows(cc[16:32])])
        if first:
            wait(g_uv)
        ctx = [None, None]
        if first:
            for cb in range(NCB - 1):
                xblock(srcs[cb], wuv_u, cb, ctx, XM)
            xblock(srcs[NCB - 1], wuv_u, NCB - 1, ctx, XM, hhs=(0,))
            xblock(srcs[NCB - 1], wuv_u, NCB - 1, ctx, XM, hhs=(1,))
            return ctx, []
        for cb in range(NCB):
            xblock(srcs[cb], wuv_u, cb, ctx, XM, hhs=(0,))

        def e_tile(cb, r):
            def fn():
                o = _dot(xlhs(srcs[cb][1], r, XM), xtile(wuv_u, 16 * cb + r, 1))
                ctx[1] = _acc(ctx[1], o)
                return o[0:8]
            return fn
        return ctx, [e_tile(cb, r) for cb in range(NCB) for r in range(16)]

    def h_last_lhs(hl):
        z = jnp.zeros_like(hl)
        ev = jnp.where(lane < 64, hl, z)
        od = jnp.where(lane < 64, z, hl)
        return _rep16(jnp.where(sub % 2 == 0, ev, od))

    def h_last_tile(L, mb, mb2):
        r0 = NFB * 64
        t = jnp.concatenate([wd_u[pl.ds(mb * (F // 2) + r0, 32), :], wd_u[pl.ds(mb2 * (F // 2) + r0, 32), :]],
                            axis=0)
        return _dot(L, pltpu.bitcast(t, BF))[0:8]

    def mix(x, ctx, e_fns, first):
        if first:
            wait(g_g)
            transpose_gu(0, wg)
            wait(g_u)
            transpose_gu(1, wu)
            transpose_gu_last()
            ones = jnp.ones((16, 128), BF)
            for n in range(2 * NFB + 1):
                a = None
                for mb in range(NMB):
                    a = _acc(a, _dot(ones, _tile(guT_u, (n * NMB + mb) * 64))[0:8])
                cs_scr[pl.ds(n * 8, 8), :] = a
            wait(g_o1)

        def flhs(h):
            hh, r = divmod(h, 16)
            return jnp.broadcast_to(ctx[hh][r:r + 1, :], (16, 128)).astype(BF)
        acc = [None] * NMB
        vacc_f = [None] * NMB
        mts, Lf = {}, {}

        def f_tile(h, mb):
            def fn():
                if h not in Lf:
                    Lf[h] = flhs(h)
                acc[mb] = _acc(acc[mb], _dot(Lf[h], _tile(wo_u, mb * (SK // 2) + h * 64))[0:8])
                return acc[mb]
            return fn

        def f_group(h, k):
            def fn(dep):
                if h not in mts:
                    mts[h] = _col_multipliers(flhs(h))
                mlo, mhi = _unpack(tie(mts[h][8 * k:8 * k + 8], dep))
                for mb in range(NMB):
                    wlo, whi = _unpack(wo_u[pl.ds(mb * (SK // 2) + h * 64 + 8 * k, 8), :])
                    vacc_f[mb] = _acc(vacc_f[mb], wlo * mlo + whi * mhi)
            return fn
        paced(list(e_fns) + [f_tile(h, mb) for h in range(NH1) if h not in FV for mb in range(NMB)],
              [f_group(h, k) for h in FV for k in range(8)], 1, 1.0, 40 if e_fns else 0)
        if first:
            wait(g_o2)
        Ls = {h: flhs(h) for h in range(NH1, H)}
        x1 = []
        for mb in range(NMB):
            for h in Ls:
                acc[mb] = _acc(acc[mb], _dot(Ls[h], _tile(wo_u, mb * (SK // 2) + h * 64))[0:8])
            x1.append(x[mb] + (acc[mb] + jnp.sum(vacc_f[mb], axis=0, keepdims=True)))

        L = [_rep16(x1[b]) for b in range(NMB)]
        mean, inv = _stats(x1)
        xn1 = [(x1[b] - mean) * inv for b in range(NMB)]
        rr = xn1[0] * wr_rows[0]
        for b in range(1, NMB):
            rr = rr + xn1[b] * wr_rows[b]
        r = jnp.sum(rr, axis=1, keepdims=True)
        sig = 1.0 / (1.0 + jnp.exp(-r))

        def fin(a, n):
            return (a - mean * cs_scr[pl.ds(n * 8, 8), :]) * inv
        hs = [None] * (NFB + 1)
        accs, ndone = {}, {}
        mfb = [fb for fb in range(NFB) if fb not in GV]

        def g_tile(fb, which, mb):
            def fn():
                o = _dot(L[mb], _tile(guT_u, gu_index(which, fb, mb) * 64))[0:8]
                ndone[fb] = ndone.get(fb, 0) + 1
                accs[fb, which] = _acc(accs.get((fb, which)), o)
                return accs[fb, which]
            return fn
        mxu_fns = [g_tile(fb, which, mb) for mb in range(NMB) for fb in mfb[:G1] for which in range(2)]
        mxu_fns += [g_tile(fb, which, mb) for fb in mfb[G1:] for which in range(2) for mb in range(NMB)]
        vacc_g, mtg = {}, {}

        def g_group(mb, k, which):
            def fn(dep):
                if mb not in mtg:
                    mtg[mb] = _col_multipliers(_rep16(x1[mb]))
                mlo, mhi = _unpack(tie(mtg[mb][8 * k:8 * k + 8], dep))
                for fb in GV:
                    wlo, whi = _unpack(guT_u[pl.ds(gu_index(which, fb, mb) * 64 + 8 * k, 8), :])
                    vacc_g[fb, which] = _acc(vacc_g.get((fb, which)), wlo * mlo + whi * mhi)
            return fn
        vpu_fns = [g_group(mb, k, which) for mb in range(NMB) for k in range(8) for which in range(2)]
        lastacc = [None]

        def gl_tile(mb):
            def fn():
                lastacc[0] = _acc(lastacc[0], _dot(L[mb], _tile(guT_u, (2 * NFB * NMB + mb) * 64))[0:8])
                res = lastacc[0]
                if mb == NMB - 1:
                    a = fin(res, 2 * NFB)
                    sw = pltpu.roll(a, 64, axis=1)
                    g = jnp.where(lane < 64, a, sw)
                    u = jnp.where(lane < 64, sw, a)
                    hs[NFB] = _silu(g) * u
                return res
            return fn
        mxu_fns += [gl_tile(mb) for mb in range(NMB)]

        def finish_block(fb):
            if hs[fb] is None:
                assert ndone[fb] == 2 * NMB
                hs[fb] = _silu(fin(accs[fb, 0], fb)) * fin(accs[fb, 1], NFB + fb)

        def finish_vpu_blocks():
            for fb in GV:
                gu = [fin(jnp.sum(vacc_g[fb, which], axis=0, keepdims=True), which * NFB + fb)
                      for which in range(2)]
                hs[fb] = _silu(gu[0]) * gu[1]
        if first:
            paced(mxu_fns, vpu_fns, 2, 1.1, 0)
            for fb in mfb:
                finish_block(fb)
            finish_vpu_blocks()
            return x1, xn1, sig, hs, mean

        yacc = [None] * NMB
        Lh = {}

        def h_tile(fb, mb):
            def fn():
                if fb not in Lh:
                    if fb not in GV:
                        finish_block(fb)
                    Lh[fb] = _rep16(hs[fb])
                yacc[mb] = _acc(yacc[mb], _dot(Lh[fb], _tile(wd_u, mb * (F // 2) + fb * 64))[0:8])
                return yacc[mb]
            return fn

        def h_last(mb):
            def fn():
                if NFB not in Lh:
                    Lh[NFB] = h_last_lhs(hs[NFB])
                mb2 = min(mb + 1, NMB - 1)
                o = h_last_tile(Lh[NFB], mb, mb2)
                yacc[mb] = yacc[mb] + jnp.broadcast_to(o[0:1], (8, 128))
                if mb2 != mb:
                    yacc[mb2] = yacc[mb2] + jnp.broadcast_to(o[1:2], (8, 128))
                return yacc[mb]
            return fn
        for fb in mfb + [NFB] + list(GV):
            if fb == NFB:
                mxu_fns += [h_last(mb) for mb in range(0, NMB, 2)]
            elif fb not in HV:
                mxu_fns += [h_tile(fb, mb) for mb in range(NMB)]
        vacc_h, mth = [None] * NMB, {}

        def h_group(fb, k):
            def fn(dep):
                if fb not in mth:
                    finish_block(fb)
                    mth[fb] = _col_multipliers(_rep16(hs[fb]))
                mlo, mhi = _unpack(tie(mth[fb][8 * k:8 * k + 8], dep))
                for mb in range(NMB):
                    wlo, whi = _unpack(wd_u[pl.ds(mb * (F // 2) + fb * 64 + 8 * k, 8), :])
                    vacc_h[mb] = _acc(vacc_h[mb], wlo * mlo + whi * mhi)
            return fn
        last_g = vpu_fns[-1]

        def last_g_group(dep):
            last_g(dep)
            finish_vpu_blocks()
        vpu_fns[-1] = last_g_group
        vpu_fns += [h_group(fb, k) for fb in HV for k in range(8)]
        paced(mxu_fns, vpu_fns, 2, 1.1, 0)
        y = [yacc[mb] + jnp.sum(vacc_h[mb], axis=0, keepdims=True) for mb in range(NMB)]
        return x1, xn1, sig, y, None

    def next_layer_head(x1, xn1, sig, hs, mean1):
        Lh = [_rep16(hs[fb]) for fb in range(NFB)]
        Ll = h_last_lhs(hs[NFB])
        acc = [None] * NMB
        x2 = [None] * NMB
        q = [None, None]
        ds = {}

        def hpart(fbs, mbs):
            for fb in fbs:
                for mb in mbs:
                    acc[mb] = _acc(acc[mb], _dot(Lh[fb], _tile(wd_u, mb * (F // 2) + fb * 64))[0:8])

        def hlast(mb, mb2):
            o = h_last_tile(Ll, mb, mb2)
            acc[mb] = acc[mb] + jnp.broadcast_to(o[0:1], (8, 128))
            if mb2 != mb:
                acc[mb2] = acc[mb2] + jnp.broadcast_to(o[1:2], (8, 128))

        def finish_x(mb):
            x2[mb] = x1[mb] + xn1[mb] + acc[mb] * sig
            ds[mb] = dup_bits(x2[mb])

        def ablock(mb, rs):
            xblock([ds[mb], ds[mb]], wq_u, mb, q, XQ, rs=rs)

        wait(g_d012)
        hpart(range(NFB), (0, 1))
        hlast(0, 1)
        hpart(range(NFB), (2,))
        hlast(2, 2)
        finish_x(0)
        finish_x(1)
        ablock(0, range(16))
        finish_x(2)
        ablock(1, range(16))
        ablock(2, range(16 - NCOV))
        wait(g_d34a)
        hpart(range(FS34), (3, 4))
        wait(g_d34b)
        hpart(range(FS34, NFB), (3, 4))
        hlast(3, 4)
        st = []

        def a_tile(blk, r, hh):
            def fn():
                l0 = xlhs(ds[blk], r, XQ)
                if blk == NMB - 1 and hh == 0 and r == 8:
                    l0 = pltpu.bitcast(tie(pltpu.bitcast(l0, U32), jnp.broadcast_to(st[0][1], (8, 128))), BF)
                o = _dot(l0, xtile(wq_u, 16 * blk + r, hh))
                q[hh] = _acc(q[hh], o)
                return o[0:8]
            return fn
        for r in range(16 - NCOV, 16):
            a_tile(2, r, 0)()
            a_tile(2, r, 1)()
        finish_x(3)
        finish_x(4)
        st.append(_stats_shift(x2, mean1))
        for blk in (3, 4):
            for r in range(16):
                a_tile(blk, r, 0)()
        return x2, q, [a_tile(blk, r, 1) for blk in (3, 4) for r in range(16)], st[0]

    wait(g_q)
    xrow = xb[0].astype(F32)
    x = [jnp.broadcast_to(xrow[:, b * 128:(b + 1) * 128], (8, 128)) for b in range(NMB)]
    wrf = wrb[...].astype(F32)
    wr_rows = [jnp.broadcast_to(wrf[b:b + 1, :], (8, 128)) for b in range(NMB)]
    always = (pltpu.bitcast(wr_rows[0], U32) | np.uint32(1)) != np.uint32(0)
    csq = colsum_q()
    q = [None, None]
    for mb in range(NMB):
        d = dup_bits(x[mb])
        xblock([d, d], wq_u, mb, q, XQ)
    st = _stats(x)
    wait(g_uk)
    relayout_uk()
    ctx, e_fns = attention(q, st, csq, True)
    x1, xn1, sig, hs, mean1 = mix(x, ctx, e_fns, True)
    x, q, a_fns, st = next_layer_head(x1, xn1, sig, hs, mean1)
    ctx, e_fns = attention(q, st, csq, False, a_fns)
    x1, xn1, sig, y, _ = mix(x, ctx, e_fns, False)
    xo = [x1[b] + xn1[b] + y[b] * sig for b in range(NMB)]
    out = jnp.concatenate([xb_[0:1] for xb_ in xo], axis=1)
    o_ref[...] = out.astype(BF).reshape(1, 1, M)


def _call(A_x, A_c_kv, A_w_q, A_w_uk, A_w_uv, A_w_o, B_w_r, B_w_gate, B_w_up, B_w_down):
    scratch = [
        pltpu.VMEM((1, 1, M), BF),
        pltpu.VMEM((NMB, 128), BF),
        pltpu.VMEM((M * H, D), BF),
        pltpu.VMEM((DC * H, D), BF),
        pltpu.VMEM((DC * H, D), BF),
        pltpu.VMEM((NCB * SK, 128), BF),
        pltpu.VMEM((NCB * SK, 128), BF),
        pltpu.VMEM((DC * H, D), BF),
        pltpu.VMEM((NMB * SK, 128), BF),
        pltpu.VMEM((F, M), BF),
        pltpu.VMEM((F, M), BF),
        pltpu.VMEM(((2 * NFB * NMB + NMB) * 128, 128), BF),
        pltpu.VMEM((NMB * F, 128), BF),
        pltpu.VMEM((H, SK), F32),
        pltpu.VMEM(((2 * NFB + 1) * 8, 128), F32),
        pltpu.SemaphoreType.DMA((NSEM,)),
    ]
    return pl.pallas_call(
        _kernel,
        out_shape=jax.ShapeDtypeStruct((1, 1, M), BF),
        in_specs=[pl.BlockSpec(memory_space=pltpu.HBM)] * 10,
        out_specs=pl.BlockSpec(memory_space=pltpu.VMEM),
        scratch_shapes=scratch,
        compiler_params=pltpu.CompilerParams(vmem_limit_bytes=100 * 1024 * 1024),
    )(A_x, B_w_r.reshape(NMB, 128), A_w_q.reshape(M * H, D), A_w_uk.reshape(DC * H, D),
      A_c_kv.reshape(SK, DC), A_w_uv.reshape(DC * H, D), A_w_o.reshape(H * D, M),
      B_w_gate.T, B_w_up.T, B_w_down)


@jax.jit
def pallas_interleave_layers__compressed_kv_cla__moe_arch_mod__decode_kernel(
    A_x: jax.Array,
    A_c_kv: jax.Array,
    A_w_q: jax.Array,
    A_w_uk: jax.Array,
    A_w_uv: jax.Array,
    A_w_o: jax.Array,
    B_x: jax.Array,
    B_w_r: jax.Array,
    B_w_gate: jax.Array,
    B_w_up: jax.Array,
    B_w_down: jax.Array,
):
    return _call(A_x, A_c_kv, A_w_q, A_w_uk, A_w_uv, A_w_o, B_w_r, B_w_gate, B_w_up, B_w_down)
```
